```python
import os as _os
_os.environ.setdefault("JAX_PLATFORMS", "cpu")
import jax
import jax.numpy as jnp

def _softmax(x, axis=-1):
    return jax.nn.softmax(x, axis=axis)
def _gelu(x):
    return jax.nn.gelu(x, approximate=True)
def _silu(x):
    return jax.nn.silu(x)
def _sigmoid(x):
    return jax.nn.sigmoid(x)
def _layernorm(x, axis=-1, eps=1e-5):
    m = jnp.mean(x, axis=axis, keepdims=True)
    v = jnp.var(x, axis=axis, keepdims=True)
    return (x - m) / jnp.sqrt(v + eps)
def _scatter_add(tgt, idx, src, axis=0):
    return tgt.at[idx].add(src)
def _segment_sum(src, seg, n):
    return jax.ops.segment_sum(src, seg, n)
class _Rng:
    def __init__(self, key):
        self._k = key
    def _next(self):
        self._k, sub = jax.random.split(self._k)
        return sub
    def normal(self, shape):
        return jax.random.normal(self._next(), shape, dtype=jnp.bfloat16)
    def randint(self, lo, hi, shape):
        return jax.random.randint(self._next(), shape, lo, hi, dtype=jnp.int32)
    def uniform(self, shape, lo=0.0, hi=1.0):
        return jax.random.uniform(self._next(), shape, jnp.bfloat16, lo, hi)
    def permutation(self, n):
        return jax.random.permutation(self._next(), n)


kernel_name = 'sequential_preLN__mha_block__moe_arch_mod__prompt'

def setup_inputs():
    _rng = _Rng(jax.random.key(int.from_bytes(__import__("os").urandom(4), "little")))
    _w = (lambda a: (lambda t: t.astype(jnp.bfloat16) if jnp.issubdtype(t.dtype, jnp.floating) else t)(jnp.asarray(a)))
    def _A_setup():
        B, S, D, H = 1, 2048, 512, 32
        return {
            "x": _w((lambda *s: _rng.normal(s) * 0.05)(B, S, D)),
            "wqkv": _w((lambda *s: _rng.normal(s) * 0.05)(D, 3 * D)),
            "wo": _w((lambda *s: _rng.normal(s) * 0.05)(D, D)),
        }
    _A_in = _A_setup()

    def _B_setup():
        B, S, D, F, C = 1, 2048, 512, 1792, 2
        return {
            "x": _w((lambda *s: _rng.normal(s) * 0.05)(B, S, D)),
            "w_r": _w((lambda *s: _rng.normal(s) * 0.05)(D)),
            "w_gate": _w((lambda *s: _rng.normal(s) * 0.05)(D, F)),
            "w_up": _w((lambda *s: _rng.normal(s) * 0.05)(D, F)),
            "w_down": _w((lambda *s: _rng.normal(s) * 0.05)(F, D)),
        }
    _B_in = _B_setup()

    return {
        "A_x": _A_in["x"],
        "A_wqkv": _A_in["wqkv"],
        "A_wo": _A_in["wo"],
        "B_x": _B_in["x"],
        "B_w_r": _B_in["w_r"],
        "B_w_gate": _B_in["w_gate"],
        "B_w_up": _B_in["w_up"],
        "B_w_down": _B_in["w_down"],
    }

def reference(A_x, A_wqkv, A_wo, B_x, B_w_r, B_w_gate, B_w_up, B_w_down):
    def _A_ref(x, wqkv, wo):
        B, S, D = x.shape
        H = 32
        Dh = D // H
        qkv = (lambda x, *d: x.transpose(*d))((x @ wqkv).reshape(B, S, 3, H, Dh), 2, 0, 3, 1, 4)
        q, k, v = qkv[0], qkv[1], qkv[2]
        scores = jnp.einsum("bhqd,bhkd->bhqk", q, k) * (Dh ** -0.5)
        p = _softmax(scores, axis=-1)
        o = jnp.einsum("bhqk,bhkd->bhqd", p, v)
        return (lambda x, *d: x.transpose(*d))(o, 0, 2, 1, 3).reshape(B, S, D) @ wo

    def _B_ref(x, w_r, w_gate, w_up, w_down):
        B, S, D = x.shape
        C = 2
        r = x @ w_r
        idx = jnp.argsort(-r, axis=-1)[:, :C]
        idx_e = jnp.repeat(idx.reshape(B, C, 1), D, axis=2)
        x_sel = jnp.take_along_axis(x, idx_e, axis=1)
        g = _silu(x_sel @ w_gate)
        u = x_sel @ w_up
        y = (g * u) @ w_down
        r_sel = _sigmoid(jnp.take_along_axis(r, idx, axis=1))
        y = y * r_sel.reshape(B, C, 1)
        b_off = (jnp.arange(B) * S).reshape(B, 1)
        flat_idx = (idx + b_off).reshape(B * C)
        zero = (x * 0.0).reshape(B * S, D)
        upd = _scatter_add(zero, flat_idx, y.reshape(B * C, D), axis=0)
        return x + upd.reshape(B, S, D)

    x = A_x
    h = x + _A_ref(_layernorm(x, axis=-1), A_wqkv, A_wo)
    h2 = h + _B_ref(_layernorm(h, axis=-1), B_w_r, B_w_gate, B_w_up, B_w_down)
    return h2
```

```python
import math

import jax
import jax.numpy as jnp
from jax import lax
import jax.experimental.pallas as pl
import jax.experimental.pallas.tpu as pltpu

S = 2048
D = 512
H = 32
DH = D // H
F = 1792
EPS = 1e-5
GH = 128 // DH
NG = H // GH
TQ = 512
NQ = S // TQ
CK = 128
NC = S // CK
LAG = 2
RB = 512
NRB = S // RB
SLAB = 16

QSCALE = (DH ** -0.5) * math.log2(math.e)
SCORE_LIMIT = 96.0
V_LIMIT = 2.0 ** 20

F32 = jnp.float32
BF16 = jnp.bfloat16
NT = (((1,), (1,)), ((), ()))
TN = (((0,), (0,)), ((), ()))


def _layernorm(x):
    m = jnp.mean(x, axis=-1, keepdims=True)
    xc = x - m
    v = jnp.mean(xc * xc, axis=-1, keepdims=True)
    return xc * lax.rsqrt(v + EPS)


def _kernel(x_hbm, wqkv_hbm, wo_hbm, wr_hbm, wg_hbm, wu_hbm, wd_hbm, out_hbm,
            x_v, wqkv_v, wo_v, wr_v, wg_v, wu_v, wd_v,
            wqvt_v, k_v, qt_v, vt_v, ot_v, h_v, hn_v, out_v, r_v, s_v, slab_v,
            in_sems, out_sems, patch_sems):
    def x_copy(b):
        rows = pl.ds(b * RB, RB)
        return pltpu.make_async_copy(x_hbm.at[rows, :], x_v.at[rows, :], in_sems.at[b])

    def w_copy(part):
        cols = pl.ds(part * D, D)
        return pltpu.make_async_copy(
            wqkv_hbm.at[:, cols], wqkv_v.at[:, cols], in_sems.at[NRB + part])

    wo_copy = pltpu.make_async_copy(wo_hbm, wo_v, in_sems.at[NRB + 3])
    wr_copy = pltpu.make_async_copy(wr_hbm, wr_v, in_sems.at[NRB + 4])
    wg_copy = pltpu.make_async_copy(wg_hbm, wg_v, in_sems.at[NRB + 5])
    wu_copy = pltpu.make_async_copy(wu_hbm, wu_v, in_sems.at[NRB + 6])
    wd_copy = pltpu.make_async_copy(wd_hbm, wd_v, in_sems.at[NRB + 7])

    x_copy(0).start()
    w_copy(1).start()
    w_copy(0).start()
    w_copy(2).start()
    for b in range(1, NRB):
        x_copy(b).start()
    wo_copy.start()
    wr_copy.start()

    x_copy(0).wait()
    xn = _layernorm(x_v[pl.ds(0, RB), :].astype(F32)).astype(BF16)
    w_copy(1).wait()
    w_copy(0).wait()
    w_copy(2).wait()
    wqvt_v[pl.ds(0, D), :] = wqkv_v[:, pl.ds(0, D)].T
    wqvt_v[pl.ds(D, D), :] = wqkv_v[:, pl.ds(2 * D, D)].T

    kabs = None
    vabs = None
    qsum = None
    for b in range(NRB):
        rows = pl.ds(b * RB, RB)
        kk = jnp.dot(xn, wqkv_v[:, pl.ds(D, D)], preferred_element_type=F32)
        qv = lax.dot_general(wqvt_v[...], xn, NT, preferred_element_type=F32)
        if b + 1 < NRB:
            x_copy(b + 1).wait()
            xn = _layernorm(x_v[pl.ds((b + 1) * RB, RB), :].astype(F32)).astype(BF16)
        for g in range(NG):
            k_v[g, rows, :] = kk[:, g * 128:(g + 1) * 128].astype(BF16)
        qt = qv[:D] * QSCALE
        vt = qv[D:]
        qt_v[:, rows] = qt.astype(BF16)
        vt_v[:, rows] = vt.astype(BF16)
        ka = jnp.max(jnp.abs(kk).reshape(RB // 8, 8, D), axis=0)
        va = jnp.max(jnp.abs(vt).reshape(D // 8, 8, RB), axis=0)
        qs = jnp.sum(jnp.abs(qt).reshape(H, DH, RB), axis=1)
        kabs = ka if kabs is None else jnp.maximum(kabs, ka)
        vabs = va if vabs is None else jnp.maximum(vabs, va)
        qsum = qs if qsum is None else jnp.maximum(qsum, qs)

    wg_copy.start()
    wu_copy.start()
    wd_copy.start()

    bound = jnp.max(qsum) * jnp.max(kabs) * 1.02
    fast = jnp.logical_and(bound <= SCORE_LIMIT, jnp.max(vabs) <= V_LIMIT)

    row_head = lax.broadcasted_iota(jnp.int32, (128, TQ), 0) // DH

    def fast_group(g, cols):
        qt = qt_v[pl.ds(pl.multiple_of(g * 128, 128), 128), cols]
        st = {}

        def stage_a(j, c):
            if c == 0:
                st[j] = dict(w=jnp.where(row_head == j, qt, jnp.zeros_like(qt)))
            s = jnp.dot(k_v[g, pl.ds(c * CK, CK), :], st[j]['w'],
                        preferred_element_type=F32)
            p = jnp.exp2(s)
            lc = jnp.sum(p.reshape(CK // 8, 8, TQ), axis=0)
            st[j]['l'] = lc if c == 0 else st[j]['l'] + lc
            return p.astype(BF16)

        def stage_b(j, c, p):
            hrows = pl.ds(pl.multiple_of(g * 128 + j * DH, DH), DH)
            oc = jnp.dot(vt_v[hrows, pl.ds(c * CK, CK)], p, preferred_element_type=F32)
            st[j]['o'] = oc if c == 0 else st[j]['o'] + oc
            if c == NC - 1:
                lsum = jnp.sum(st[j]['l'], axis=0, keepdims=True)
                ot_v[hrows, :] = (st[j]['o'] / lsum).astype(BF16)

        seq = [(j, c) for j in range(GH) for c in range(NC)]
        ps = {}
        for t in range(len(seq) + LAG):
            if t < len(seq):
                ps[t] = stage_a(*seq[t])
            if t >= LAG:
                stage_b(*seq[t - LAG], ps.pop(t - LAG))

    def slow_head(h, cols):
        g = h // GH
        qt = qt_v[pl.ds(pl.multiple_of(g * 128, 128), 128), cols]
        w = jnp.where(row_head == h % GH, qt, jnp.zeros_like(qt))
        hrows = pl.ds(pl.multiple_of(h * DH, DH), DH)
        m = None
        for c in range(S // 512):
            s = jnp.dot(k_v[g, pl.ds(c * 512, 512), :], w, preferred_element_type=F32)
            s_v[pl.ds(c * 512, 512), :] = s
            mc = jnp.max(s.reshape(512 // 8, 8, TQ), axis=0)
            m = mc if m is None else jnp.maximum(m, mc)
        m = jnp.max(m, axis=0, keepdims=True)
        l = None
        o = None
        for c in range(S // 512):
            p = jnp.exp2(s_v[pl.ds(c * 512, 512), :] - m)
            lc = jnp.sum(p.reshape(512 // 8, 8, TQ), axis=0)
            oc = jnp.dot(vt_v[hrows, pl.ds(c * 512, 512)], p.astype(BF16),
                         preferred_element_type=F32)
            l = lc if l is None else l + lc
            o = oc if o is None else o + oc
        lsum = jnp.sum(l, axis=0, keepdims=True)
        ot_v[hrows, :] = (o / lsum).astype(BF16)

    def out_copy(qb):
        rows = pl.ds(pl.multiple_of(qb * TQ, TQ), TQ)
        return pltpu.make_async_copy(out_v.at[rows, :], out_hbm.at[rows, :],
                                     out_sems.at[qb])

    wo_copy.wait()
    wr_copy.wait()

    def q_block(qb, carry):
        cols = pl.ds(pl.multiple_of(qb * TQ, TQ), TQ)

        @pl.when(fast)
        def _():
            def body(g, c):
                fast_group(g, cols)
                return c
            lax.fori_loop(0, NG, body, 0)

        @pl.when(jnp.logical_not(fast))
        def _():
            def body(h, c):
                slow_head(h, cols)
                return c
            lax.fori_loop(0, H, body, 0)

        attn = lax.dot_general(ot_v[...], wo_v[...], TN, preferred_element_type=F32)
        h = x_v[cols, :].astype(F32) + attn
        hn = _layernorm(h)
        h_v[cols, :] = h
        hn_v[cols, :] = hn
        out_v[cols, :] = (h + hn).astype(BF16)
        out_copy(qb).start()
        wr16 = jnp.broadcast_to(wr_v[...], (16, D))
        r = lax.dot_general(wr16, hn.astype(BF16), NT, preferred_element_type=F32)
        r_v[:, cols] = r[:8]
        return carry

    lax.fori_loop(0, NQ, q_block, 0)

    r = r_v[...]
    pos = lax.broadcasted_iota(jnp.int32, (8, S), 1)
    m1 = jnp.max(r)
    i1 = jnp.minimum(jnp.min(jnp.where(r == m1, pos, S)), S - 1)
    r2 = jnp.where(pos == i1, -jnp.inf, r)
    m2 = jnp.max(r2)
    i2 = jnp.minimum(jnp.min(jnp.where(r2 == m2, pos, S)), S - 1)

    row16 = lax.broadcasted_iota(jnp.int32, (SLAB, D), 0)
    xs = jnp.where(row16 == 0, hn_v[pl.ds(i1, 1), :], hn_v[pl.ds(i2, 1), :]).astype(BF16)
    wg_copy.wait()
    wu_copy.wait()
    wd_copy.wait()
    gate = jnp.dot(xs, wg_v[...], preferred_element_type=F32)
    up = jnp.dot(xs, wu_v[...], preferred_element_type=F32)
    act = (gate * jax.nn.sigmoid(gate) * up).astype(BF16)
    y = jnp.dot(act, wd_v[...], preferred_element_type=F32)
    y = y * jax.nn.sigmoid(jnp.where(row16 == 0, m1, m2))
    y1 = y[0:1]
    y2 = y[1:2]

    for qb in range(NQ):
        out_copy(qb).wait()

    def patch(slot, idx):
        base = pl.multiple_of((idx // SLAB) * SLAB, SLAB)
        rows = pl.ds(base, SLAB)
        rid = row16 + base
        upd = jnp.where(rid == i1, y1, 0.0) + jnp.where(rid == i2, y2, 0.0)
        slab_v[slot] = (h_v[rows, :] + (hn_v[rows, :] + upd)).astype(BF16)
        return pltpu.make_async_copy(slab_v.at[slot], out_hbm.at[rows, :],
                                     patch_sems.at[slot])

    cp1 = patch(0, i1)
    cp1.start()

    @pl.when(i1 // SLAB != i2 // SLAB)
    def _():
        cp2 = patch(1, i2)
        cp2.start()
        cp2.wait()

    cp1.wait()


@jax.jit
def pallas_sequential_preLN__mha_block__moe_arch_mod__prompt_kernel(
    A_x: jax.Array,
    A_wqkv: jax.Array,
    A_wo: jax.Array,
    B_x: jax.Array,
    B_w_r: jax.Array,
    B_w_gate: jax.Array,
    B_w_up: jax.Array,
    B_w_down: jax.Array,
):
    del B_x
    any_spec = pl.BlockSpec(memory_space=pl.ANY)
    out = pl.pallas_call(
        _kernel,
        out_shape=jax.ShapeDtypeStruct((S, D), BF16),
        in_specs=[any_spec] * 7,
        out_specs=any_spec,
        scratch_shapes=[
            pltpu.VMEM((S, D), BF16),
            pltpu.VMEM((D, 3 * D), BF16),
            pltpu.VMEM((D, D), BF16),
            pltpu.VMEM((1, D), BF16),
            pltpu.VMEM((D, F), BF16),
            pltpu.VMEM((D, F), BF16),
            pltpu.VMEM((F, D), BF16),
            pltpu.VMEM((2 * D, D), BF16),
            pltpu.VMEM((NG, S, 128), BF16),
            pltpu.VMEM((D, S), BF16),
            pltpu.VMEM((D, S), BF16),
            pltpu.VMEM((D, TQ), BF16),
            pltpu.VMEM((S, D), F32),
            pltpu.VMEM((S, D), F32),
            pltpu.VMEM((S, D), BF16),
            pltpu.VMEM((8, S), F32),
            pltpu.VMEM((S, TQ), F32),
            pltpu.VMEM((2, SLAB, D), BF16),
            pltpu.SemaphoreType.DMA((NRB + 8,)),
            pltpu.SemaphoreType.DMA((NQ,)),
            pltpu.SemaphoreType.DMA((2,)),
        ],
        compiler_params=pltpu.CompilerParams(vmem_limit_bytes=100 * 1024 * 1024),
    )(A_x.reshape(S, D), A_wqkv, A_wo, B_w_r.reshape(1, D), B_w_gate, B_w_up, B_w_down)
    return out.reshape(1, S, D)
```

```python
import math

import jax
import jax.numpy as jnp
from jax import lax
import jax.experimental.pallas as pl
import jax.experimental.pallas.tpu as pltpu

S = 2048
D = 512
H = 32
DH = D // H
F = 1792
EPS = 1e-5
GH = 128 // DH
NG = H // GH
TQ = 512
NQ = S // TQ
NIT = NQ * NG
CK = 128
NC = S // CK
LAG = 2
RB = 512
NRB = S // RB
PR = 128
NP = S // PR
PLAG = NG + 1
SLAB = 16
NV = 16
NM = CK - NV
NB = TQ // 128
NCB = S // 128

QSCALE = (DH ** -0.5) * math.log2(math.e)
SCORE_LIMIT = 96.0
V_LIMIT = 2.0 ** 20

F32 = jnp.float32
BF16 = jnp.bfloat16
NT = (((1,), (1,)), ((), ()))


def _layernorm(x):
    m = jnp.mean(x, axis=-1, keepdims=True)
    xc = x - m
    v = jnp.mean(xc * xc, axis=-1, keepdims=True)
    return xc * lax.rsqrt(v + EPS)


def _kernel(x_hbm, wqkv_hbm, wo_hbm, wr_hbm, wg_hbm, wu_hbm, wd_hbm, out_hbm,
            kb_v, q32_v, k32_v, x_v, wqkv_v, wo_v, wr_v, wg_v, wu_v, wd_v,
            xn_v, wqvt_v, k_v, qt_v, vt_v, ot_v, h_v, hn_v, out_v, r_v, s_v, slab_v,
            in_sems, out_sems, patch_sems):
    def x_copy(b):
        rows = pl.ds(b * RB, RB)
        return pltpu.make_async_copy(x_hbm.at[rows, :], x_v.at[rows, :], in_sems.at[b])

    def w_copy(part):
        cols = pl.ds(part * D, D)
        return pltpu.make_async_copy(
            wqkv_hbm.at[:, cols], wqkv_v.at[:, cols], in_sems.at[NRB + part])

    wo_copy = pltpu.make_async_copy(wo_hbm, wo_v, in_sems.at[NRB + 3])
    wr_copy = pltpu.make_async_copy(wr_hbm, wr_v, in_sems.at[NRB + 4])
    wg_copy = pltpu.make_async_copy(wg_hbm, wg_v, in_sems.at[NRB + 5])
    wu_copy = pltpu.make_async_copy(wu_hbm, wu_v, in_sems.at[NRB + 6])
    wd_copy = pltpu.make_async_copy(wd_hbm, wd_v, in_sems.at[NRB + 7])

    x_copy(0).start()
    w_copy(1).start()
    for b in range(1, NRB):
        x_copy(b).start()
    w_copy(0).start()
    w_copy(2).start()
    wo_copy.start()
    wr_copy.start()

    def ln1_block(b):
        rows = pl.ds(b * RB, RB)
        xf = x_v[rows, :].astype(F32)
        h_v[rows, :] = xf
        xn_v[rows, :] = _layernorm(xf).astype(BF16)

    ot_v[...] = jnp.zeros_like(ot_v)
    x_copy(0).wait()
    ln1_block(0)
    w_copy(1).wait()

    kabs = None
    for b in range(NRB):
        rows = pl.ds(b * RB, RB)
        if b + 1 < NRB:
            x_copy(b + 1).wait()
            ln1_block(b + 1)
        else:
            w_copy(0).wait()
            w_copy(2).wait()
            wo_copy.wait()
            wr_copy.wait()
            wg_copy.start()
            wu_copy.start()
            wd_copy.start()
            wqvt_v[pl.ds(0, D), :] = wqkv_v[:, pl.ds(0, D)].T
            wqvt_v[pl.ds(D, D), :] = wqkv_v[:, pl.ds(2 * D, D)].T
        kk = jnp.dot(xn_v[rows, :], wqkv_v[:, pl.ds(D, D)], preferred_element_type=F32)
        for g in range(NG):
            k_v[g, rows, :] = kk[:, g * 128:(g + 1) * 128].astype(BF16)
            for c in range(RB // CK):
                k32_v[g, pl.ds((b * (RB // CK) + c) * NV, NV), :] = (
                    kk[c * CK + NM:(c + 1) * CK, g * 128:(g + 1) * 128])
        ka = jnp.max(jnp.abs(kk).reshape(RB // 8, 8, D), axis=0)
        kabs = ka if kabs is None else jnp.maximum(kabs, ka)

    def qv_block(b, carry):
        vabs, qsum = carry
        rows = pl.ds(pl.multiple_of(b * RB, RB), RB)
        qv = lax.dot_general(wqvt_v[...], xn_v[rows, :], NT, preferred_element_type=F32)
        qt = qv[:D] * QSCALE
        vt = qv[D:]
        qt_v[:, rows] = qt.astype(BF16)
        for cb in range(RB // 128):
            q32_v[b * (RB // 128) + cb, pl.ds(0, D), :] = qt[:, cb * 128:(cb + 1) * 128]
        vt_v[:, rows] = vt.astype(BF16)
        va = jnp.max(jnp.abs(vt).reshape(D // 8, 8, RB), axis=0)
        qs = jnp.sum(jnp.abs(qt).reshape(H, DH, RB), axis=1)
        return jnp.maximum(vabs, va), jnp.maximum(qsum, qs)

    vabs, qsum = lax.fori_loop(
        0, NRB, qv_block, (jnp.zeros((8, RB), F32), jnp.zeros((H, RB), F32)))

    bound = jnp.max(qsum) * jnp.max(kabs) * 1.02
    fast = jnp.logical_and(bound <= SCORE_LIMIT, jnp.max(vabs) <= V_LIMIT)

    def out_proj(t, o_rows, r0, nrows):
        rows = pl.ds(pl.multiple_of((t // NG) * TQ + r0, PR), nrows)
        wo_g = wo_v[pl.ds(pl.multiple_of((t % NG) * 128, 128), 128), :]
        h_v[rows, :] = h_v[rows, :] + jnp.dot(o_rows, wo_g, preferred_element_type=F32)

    def ln2_part(p):
        rows = pl.ds(pl.multiple_of(p * PR, PR), PR)
        h = h_v[rows, :]
        hn = _layernorm(h)
        hn_v[rows, :] = hn
        out_v[rows, :] = (h + hn).astype(BF16)
        t = hn * wr_v[...].astype(F32).reshape(1, D)
        t = (t[:, 0:128] + t[:, 128:256]) + (t[:, 256:384] + t[:, 384:512])
        r_v[pl.ds(p, 1), :] = jnp.sum(t.T, axis=0, keepdims=True)

    def out_copy(p):
        rows = pl.ds(pl.multiple_of(p * PR, PR), PR)
        return pltpu.make_async_copy(out_v.at[rows, :], out_hbm.at[rows, :],
                                     out_sems.at[p])

    def head_weights(g, j, cols):
        q = qt_v[pl.ds(pl.multiple_of(g * 128 + j * DH, DH), DH), cols]
        parts = []
        if j > 0:
            parts.append(jnp.zeros((j * DH, TQ), BF16))
        parts.append(q)
        if j < GH - 1:
            parts.append(jnp.zeros(((GH - 1 - j) * DH, TQ), BF16))
        return jnp.concatenate(parts, axis=0)

    def vpu_scores(t, j, c):
        g = t % NG
        res = {}
        prev = [None] * (NV // 8)
        for b in range(NB):
            cur = list(prev)
            for d in range(DH):
                qrow = q32_v[(t // NG) * NB + b,
                             pl.ds(pl.multiple_of(g * 128, 128) + j * DH + d, 8, stride=0), :]
                for r in range(NV // 8):
                    term = kb_v[g, j * DH + d, pl.ds(c * NV + r * 8, 8), :] * qrow
                    cur[r] = term if cur[r] is None else cur[r] + term
            for r in range(NV // 8):
                res[(r, b)] = cur[r] if prev[r] is None else cur[r] - prev[r]
            prev = cur
        return jnp.concatenate(
            [jnp.concatenate([res[(r, b)] for b in range(NB)], axis=1)
             for r in range(NV // 8)], axis=0)

    def fast_iter(t, offload):
        g = t % NG
        cols = pl.ds(pl.multiple_of((t // NG) * TQ, TQ), TQ)
        o_prev = ot_v[...].T
        if offload:
            ln2_part(jnp.maximum(t - PLAG, 0))
        else:
            kk = k32_v[g]
            for d in range(128):
                kb_v[g, d] = jnp.broadcast_to(kk[:, d:d + 1], (NC * NV, 128))
        nm = NM if offload else CK
        st = {}

        def stage_a(j, c):
            if c == 0:
                st[j] = dict(w=head_weights(g, j, cols))
            s = jnp.dot(k_v[g, pl.ds(c * CK, nm), :], st[j]['w'],
                        preferred_element_type=F32)
            p = jnp.exp2(s)
            lc = jnp.sum(p.reshape(nm // 8, 8, TQ), axis=0)
            if offload:
                pv = jnp.exp2(vpu_scores(t, j, c))
                lc = lc + jnp.sum(pv.reshape(NV // 8, 8, TQ), axis=0)
                p = jnp.concatenate([p, pv], axis=0)
            st[j]['l'] = lc if c == 0 else st[j]['l'] + lc
            return p.astype(BF16)

        def stage_b(j, c, p):
            hrows = pl.ds(pl.multiple_of(g * 128 + j * DH, DH), DH)
            oc = jnp.dot(vt_v[hrows, pl.ds(c * CK, CK)], p, preferred_element_type=F32)
            st[j]['o'] = oc if c == 0 else st[j]['o'] + oc
            if c == NC - 1:
                lsum = jnp.sum(st[j]['l'], axis=0, keepdims=True)
                ot_v[pl.ds(j * DH, DH), :] = (st[j]['o'] / lsum).astype(BF16)

        seq = [(j, c) for j in range(GH) for c in range(NC)]
        ps = {}
        for i in range(len(seq) + LAG):
            if i < len(seq):
                ps[i] = stage_a(*seq[i])
            if i == len(seq):
                out_proj(jnp.maximum(t - 1, 0), o_prev, 0, TQ)
            if i >= LAG:
                stage_b(*seq[i - LAG], ps.pop(i - LAG))

        if offload:
            @pl.when(t >= PLAG)
            def _():
                out_copy(t - PLAG).start()

    def fast_first(t, carry):
        fast_iter(t, False)
        return carry

    def fast_rest(t, carry):
        fast_iter(t, True)
        return carry

    def slow_iter(t, carry):
        g = t % NG
        cols = pl.ds(pl.multiple_of((t // NG) * TQ, TQ), TQ)
        out_proj(jnp.maximum(t - 1, 0), ot_v[...].T, 0, TQ)
        ln2_part(jnp.maximum(t - PLAG, 0))
        row_head = lax.broadcasted_iota(jnp.int32, (128, TQ), 0) // DH

        def head(j, c2):
            qt = qt_v[pl.ds(pl.multiple_of(g * 128, 128), 128), cols]
            w = jnp.where(row_head == j, qt, jnp.zeros_like(qt))
            hrows = pl.ds(pl.multiple_of(g * 128 + j * DH, DH), DH)
            m = None
            for c in range(S // 512):
                s = jnp.dot(k_v[g, pl.ds(c * 512, 512), :], w, preferred_element_type=F32)
                s_v[pl.ds(c * 512, 512), :] = s
                mc = jnp.max(s.reshape(512 // 8, 8, TQ), axis=0)
                m = mc if m is None else jnp.maximum(m, mc)
            m = jnp.max(m, axis=0, keepdims=True)
            l = None
            o = None
            for c in range(S // 512):
                p = jnp.exp2(s_v[pl.ds(c * 512, 512), :] - m)
                lc = jnp.sum(p.reshape(512 // 8, 8, TQ), axis=0)
                oc = jnp.dot(vt_v[hrows, pl.ds(c * 512, 512)], p.astype(BF16),
                             preferred_element_type=F32)
                l = lc if l is None else l + lc
                o = oc if o is None else o + oc
            lsum = jnp.sum(l, axis=0, keepdims=True)
            ot_v[pl.ds(pl.multiple_of(j * DH, DH), DH), :] = (o / lsum).astype(BF16)
            return c2
        lax.fori_loop(0, GH, head, 0)

        @pl.when(t >= PLAG)
        def _():
            out_copy(t - PLAG).start()
        return carry

    @pl.when(fast)
    def _():
        lax.fori_loop(0, NG, fast_first, 0)
        lax.fori_loop(NG, NIT, fast_rest, 0)

    @pl.when(jnp.logical_not(fast))
    def _():
        lax.fori_loop(0, NIT, slow_iter, 0)

    o_last = ot_v[...].T
    for p in range(NIT - PLAG, NP):
        r0 = p * PR - (NQ - 1) * TQ
        if r0 >= 0:
            out_proj(NIT - 1, o_last[r0:r0 + PR], r0, PR)
        ln2_part(p)
    for p in range(NIT - PLAG, NP):
        out_copy(p).start()

    r = r_v[...]
    pos = (lax.broadcasted_iota(jnp.int32, (NP, PR), 0) * PR
           + lax.broadcasted_iota(jnp.int32, (NP, PR), 1))
    m1 = jnp.max(r)
    i1 = jnp.minimum(jnp.min(jnp.where(r == m1, pos, S)), S - 1)
    r2 = jnp.where(pos == i1, -jnp.inf, r)
    m2 = jnp.max(r2)
    i2 = jnp.minimum(jnp.min(jnp.where(r2 == m2, pos, S)), S - 1)

    row16 = lax.broadcasted_iota(jnp.int32, (SLAB, D), 0)
    xs = jnp.where(row16 == 0, hn_v[pl.ds(i1, 1), :], hn_v[pl.ds(i2, 1), :]).astype(BF16)
    wg_copy.wait()
    wu_copy.wait()
    wd_copy.wait()
    gate = jnp.dot(xs, wg_v[...], preferred_element_type=F32)
    up = jnp.dot(xs, wu_v[...], preferred_element_type=F32)
    act = (gate * jax.nn.sigmoid(gate) * up).astype(BF16)
    y = jnp.dot(act, wd_v[...], preferred_element_type=F32)
    y = y * jax.nn.sigmoid(jnp.where(row16 == 0, m1, m2))
    y1 = y[0:1]
    y2 = y[1:2]

    for p in range(NP):
        out_copy(p).wait()

    def patch(slot, idx):
        base = pl.multiple_of((idx // SLAB) * SLAB, SLAB)
        rows = pl.ds(base, SLAB)
        rid = row16 + base
        upd = jnp.where(rid == i1, y1, 0.0) + jnp.where(rid == i2, y2, 0.0)
        slab_v[slot] = (h_v[rows, :] + (hn_v[rows, :] + upd)).astype(BF16)
        return pltpu.make_async_copy(slab_v.at[slot], out_hbm.at[rows, :],
                                     patch_sems.at[slot])

    cp1 = patch(0, i1)
    cp1.start()

    @pl.when(i1 // SLAB != i2 // SLAB)
    def _():
        cp2 = patch(1, i2)
        cp2.start()
        cp2.wait()

    cp1.wait()


@jax.jit
def pallas_sequential_preLN__mha_block__moe_arch_mod__prompt_kernel(
    A_x: jax.Array,
    A_wqkv: jax.Array,
    A_wo: jax.Array,
    B_x: jax.Array,
    B_w_r: jax.Array,
    B_w_gate: jax.Array,
    B_w_up: jax.Array,
    B_w_down: jax.Array,
):
    del B_x
    any_spec = pl.BlockSpec(memory_space=pl.ANY)
    out = pl.pallas_call(
        _kernel,
        out_shape=jax.ShapeDtypeStruct((S, D), BF16),
        in_specs=[any_spec] * 7,
        out_specs=any_spec,
        scratch_shapes=[
            pltpu.VMEM((NG, 128, NC * NV, 128), F32),
            pltpu.VMEM((NCB, D + 8, 128), F32),
            pltpu.VMEM((NG, NC * NV, 128), F32),
            pltpu.VMEM((S, D), BF16),
            pltpu.VMEM((D, 3 * D), BF16),
            pltpu.VMEM((D, D), BF16),
            pltpu.VMEM((D,), BF16),
            pltpu.VMEM((D, F), BF16),
            pltpu.VMEM((D, F), BF16),
            pltpu.VMEM((F, D), BF16),
            pltpu.VMEM((S, D), BF16),
            pltpu.VMEM((2 * D, D), BF16),
            pltpu.VMEM((NG, S, 128), BF16),
            pltpu.VMEM((D, S), BF16),
            pltpu.VMEM((D, S), BF16),
            pltpu.VMEM((128, TQ), BF16),
            pltpu.VMEM((S, D), F32),
            pltpu.VMEM((S, D), F32),
            pltpu.VMEM((S, D), BF16),
            pltpu.VMEM((NP, PR), F32),
            pltpu.VMEM((S, TQ), F32),
            pltpu.VMEM((2, SLAB, D), BF16),
            pltpu.SemaphoreType.DMA((NRB + 8,)),
            pltpu.SemaphoreType.DMA((NP,)),
            pltpu.SemaphoreType.DMA((2,)),
        ],
        compiler_params=pltpu.CompilerParams(vmem_limit_bytes=120 * 1024 * 1024),
    )(A_x.reshape(S, D), A_wqkv, A_wo, B_w_r, B_w_gate, B_w_up, B_w_down)
    return out.reshape(1, S, D)
```

```python
import math

import jax
import jax.numpy as jnp
from jax import lax
import jax.experimental.pallas as pl
import jax.experimental.pallas.tpu as pltpu

S = 2048
D = 512
H = 32
DH = D // H
F = 1792
EPS = 1e-5
GH = 128 // DH
NG = H // GH
TQ = 512
NQ = S // TQ
NB = TQ // 128
NIT = NQ * NG
CK = 128
NC = S // CK
NV = 16
NM = CK - NV
LAG = 2
XSPLIT = (0, 256, 640, 1152, S)
NXS = len(XSPLIT) - 1
WQV_STEP = 11
PR = 128
NP = S // PR
PLAG = NG + 1
OP1 = 384
SLAB = 16

QSCALE = (DH ** -0.5) * math.log2(math.e)
SCORE_LIMIT = 96.0
V_LIMIT = 2.0 ** 20

F32 = jnp.float32
BF16 = jnp.bfloat16
NN = (((1,), (0,)), ((), ()))
NT = (((1,), (1,)), ((), ()))


def _layernorm(x):
    m = jnp.mean(x, axis=-1, keepdims=True)
    xc = x - m
    v = jnp.mean(xc * xc, axis=-1, keepdims=True)
    return xc * lax.rsqrt(v + EPS)


def _kernel(x_hbm, wqkv_hbm, wo_hbm, wr_hbm, wg_hbm, wu_hbm, wd_hbm, out_hbm,
            x_v, wqkv_v, qt_v, vt_v, qb_v, kb_v, k_v, k32_v, xn_v, wqvt_v, h_v, wo_v,
            wr_v, ot_v, r_v, op_v, slab_v, wg_v, wu_v, wd_v, s_v, hn_v, out_v,
            in_sems, out_sems, patch_sems):
    def x_copy(i):
        rows = pl.ds(XSPLIT[i], XSPLIT[i + 1] - XSPLIT[i])
        return pltpu.make_async_copy(x_hbm.at[rows, :], x_v.at[rows, :], in_sems.at[i])

    def w_copy(part):
        cols = pl.ds(part * D, D)
        return pltpu.make_async_copy(
            wqkv_hbm.at[:, cols], wqkv_v.at[:, cols], in_sems.at[NXS + part])

    wo_copy = pltpu.make_async_copy(wo_hbm, wo_v, in_sems.at[NXS + 3])
    wr_copy = pltpu.make_async_copy(wr_hbm, wr_v.at[pl.ds(0, D)], in_sems.at[NXS + 4])
    wg_copy = pltpu.make_async_copy(wg_hbm, wg_v, in_sems.at[NXS + 5])
    wu_copy = pltpu.make_async_copy(wu_hbm, wu_v, in_sems.at[NXS + 6])
    wd_copy = pltpu.make_async_copy(wd_hbm, wd_v, in_sems.at[NXS + 7])

    x_copy(0).start()
    w_copy(1).start()
    for i in range(1, NXS):
        x_copy(i).start()
    w_copy(0).start()
    w_copy(2).start()
    wo_copy.start()
    wr_copy.start()

    def ln1_step(s):
        rows = pl.ds(s * CK, CK)
        xf = x_v[rows, :].astype(F32)
        h_v[rows, :] = xf
        xn = _layernorm(xf).astype(BF16)
        xn_v[rows, :] = xn
        return xn

    def k_store(s, kk, kabs):
        for g in range(NG):
            k_v[g, pl.ds(s * CK, CK), :] = kk[:, g * 128:(g + 1) * 128].astype(BF16)
            k32_v[g, pl.ds(s * NV, NV), :] = kk[:NV, g * 128:(g + 1) * 128]
        ka = jnp.max(jnp.abs(kk).reshape(CK // 8, 8, D), axis=0)
        return ka if kabs is None else jnp.maximum(kabs, ka)

    ot_v[...] = jnp.zeros_like(ot_v)
    x_copy(0).wait()
    xn = ln1_step(0)
    w_copy(1).wait()
    kabs = None
    kk_prev = None
    for s in range(NC):
        if (s + 1) * CK in XSPLIT[1:-1]:
            x_copy(XSPLIT.index((s + 1) * CK)).wait()
        if s == WQV_STEP:
            w_copy(0).wait()
            w_copy(2).wait()
            wg_copy.start()
            wu_copy.start()
            wd_copy.start()
            wqvt_v[pl.ds(0, D), :] = wqkv_v[:, pl.ds(0, D)].T
            wqvt_v[pl.ds(D, D), :] = wqkv_v[:, pl.ds(2 * D, D)].T
        if kk_prev is not None:
            kabs = k_store(s - 1, kk_prev, kabs)
        xn_next = ln1_step(s + 1) if s + 1 < NC else None
        kk_prev = jnp.dot(xn, wqkv_v[:, pl.ds(D, D)], preferred_element_type=F32)
        xn = xn_next
    kabs = k_store(NC - 1, kk_prev, kabs)

    def qv_block(b, carry):
        vabs, qsum = carry
        rows = pl.ds(pl.multiple_of(b * TQ, TQ), TQ)
        xn = xn_v[rows, :]
        qs = []
        for r0 in range(0, D, 128):
            qt = lax.dot_general(wqvt_v[pl.ds(r0, 128), :], xn, NT,
                                 preferred_element_type=F32) * QSCALE
            qt_v[pl.ds(r0, 128), rows] = qt.astype(BF16)
            qs.append(jnp.sum(jnp.abs(qt).reshape(GH, DH, TQ), axis=1))
        for jj in range(GH // NQ):
            j = b * (GH // NQ) + jj
            q0 = qt_v[pl.ds(pl.multiple_of(j * DH, DH), DH), pl.ds(0, TQ)].astype(F32)
            for cb in range(NB):
                qb_v[j, cb] = jnp.broadcast_to(
                    q0[:, None, cb * 128:(cb + 1) * 128], (DH, 8, 128))
        for r0 in range(0, D, 128):
            vt = lax.dot_general(wqvt_v[pl.ds(D + r0, 128), :], xn, NT,
                                 preferred_element_type=F32)
            vt_v[pl.ds(r0, 128), rows] = vt.astype(BF16)
            vabs = jnp.maximum(vabs, jnp.max(jnp.abs(vt).reshape(16, 8, TQ), axis=0))
        ncb = NC // NQ
        kk = k32_v[0, pl.ds(pl.multiple_of(b * ncb * NV, ncb * NV), ncb * NV), :]
        for d in range(128):
            kb_v[0, pl.ds(b * ncb, ncb), d] = jnp.broadcast_to(
                kk[:, d:d + 1], (ncb * NV, 128)).reshape(ncb, NV, 128)
        return vabs, jnp.maximum(qsum, jnp.concatenate(qs, axis=0))

    vabs, qsum = lax.fori_loop(
        0, NQ, qv_block, (jnp.zeros((8, TQ), F32), jnp.zeros((H, TQ), F32)), unroll=2)

    bound = jnp.max(qsum) * jnp.max(kabs) * 1.02
    fast = jnp.logical_and(bound <= SCORE_LIMIT, jnp.max(vabs) <= V_LIMIT)
    wo_copy.wait()
    wr_copy.wait()

    def out_proj(t, o_rows, r0, nrows):
        rows = pl.ds(pl.multiple_of((t // NG) * TQ + r0, PR), nrows)
        wo_g = wo_v[pl.ds(pl.multiple_of((t % NG) * 128, 128), 128), :]
        h_v[rows, :] = h_v[rows, :] + jnp.dot(o_rows, wo_g, preferred_element_type=F32)

    def ln2_part(p):
        rows = pl.ds(pl.multiple_of(p * PR, PR), PR)
        h = h_v[rows, :]
        hn = _layernorm(h)
        hn_v[rows, :] = hn
        out_v[rows, :] = (h + hn).astype(BF16)
        t = hn * wr_v[pl.ds(0, D)].astype(F32).reshape(1, D)
        t = (t[:, 0:128] + t[:, 128:256]) + (t[:, 256:384] + t[:, 384:512])
        r_v[pl.ds(p, 1), :] = jnp.sum(t.T, axis=0, keepdims=True)

    def out_copy(p):
        rows = pl.ds(pl.multiple_of(p * PR, PR), PR)
        return pltpu.make_async_copy(out_v.at[rows, :], out_hbm.at[rows, :],
                                     out_sems.at[p])

    def head_weights(g, j, cols):
        q = qt_v[pl.ds(pl.multiple_of(g * 128 + j * DH, DH), DH), cols]
        parts = []
        if j > 0:
            parts.append(jnp.zeros((j * DH, TQ), BF16))
        parts.append(q)
        if j < GH - 1:
            parts.append(jnp.zeros(((GH - 1 - j) * DH, TQ), BF16))
        return jnp.concatenate(parts, axis=0)

    def vpu_scores(kb, j, c):
        keys = kb[0, c, pl.ds(j * DH, DH)].reshape(DH, NV // 8, 8, 128)
        res = []
        prev = None
        for b in range(NB):
            terms = keys * qb_v[j, b][:, None]
            cur = prev
            for d in range(DH):
                cur = terms[d] if cur is None else cur + terms[d]
            res.append(cur if prev is None else cur - prev)
            prev = cur
        return jnp.concatenate(res, axis=2).reshape(NV, TQ)

    def fast_iter(t, first):
        g = t % NG
        cols = pl.ds(pl.multiple_of((t // NG) * TQ, TQ), TQ)
        o_prev = ot_v[...].T
        if first:
            kb = kb_v.at[pl.ds(g, 2)]
            kk = k32_v[g + 1]
            for d in range(128):
                kb[1, :, d] = jnp.broadcast_to(
                    kk[:, d:d + 1], (NC * NV, 128)).reshape(NC, NV, 128)
        else:
            kb = kb_v.at[pl.ds(g, 1)]
            ln2_part(jnp.maximum(t - PLAG, 0))
        st = {}

        def q_refill(j, c, tie):
            if c % 2:
                return
            js = (j - 1) % GH
            tn = t if j == 0 else jnp.minimum(t + 1, NIT - 1)
            b, d0 = c // 4, (c % 4) * 4
            qn = qt_v[pl.ds(pl.multiple_of((tn % NG) * 128 + js * DH, DH), DH),
                      pl.ds(pl.multiple_of((tn // NG) * TQ + b * 128, 128), 128)]
            qn = qn.astype(F32)[d0:d0 + 8] + tie * 0.0
            qb_v[js, b, pl.ds(d0, 8)] = jnp.broadcast_to(qn[:, None, :], (8, 8, 128))

        def stage_a(j, c):
            if c == 0:
                st[j] = dict(w=head_weights(g, j, cols))
            s = jnp.dot(k_v[g, pl.ds(c * CK + NV, NM), :], st[j]['w'],
                        preferred_element_type=F32)
            p = jnp.exp2(s)
            lc = jnp.sum(p.reshape(NM // 8, 8, TQ), axis=0)
            pv = jnp.exp2(vpu_scores(kb, j, c))
            lc = lc + jnp.sum(pv.reshape(NV // 8, 8, TQ), axis=0)
            st[j]['l'] = lc if c == 0 else st[j]['l'] + lc
            return jnp.concatenate([pv, p], axis=0)

        def stage_b(j, c, p):
            hrows = pl.ds(pl.multiple_of(g * 128 + j * DH, DH), DH)
            oc = lax.dot_general(vt_v[hrows, pl.ds(c * CK, CK)], p, NN,
                                 preferred_element_type=F32)
            q_refill(j, c, oc[:8, :128])
            st[j]['o'] = oc if c == 0 else oc + st[j]['o']
            if c == NC - 1:
                lsum = jnp.sum(st[j]['l'], axis=0, keepdims=True)
                ot_v[pl.ds(j * DH, DH), :] = (st[j]['o'] / lsum).astype(BF16)

        seq = [(j, c) for j in range(GH) for c in range(NC)]
        ps = {}
        for i in range(len(seq) + LAG):
            if i < len(seq):
                ps[i] = stage_a(*seq[i])
            if i == len(seq):
                out_proj(jnp.maximum(t - 1, 0), o_prev[:OP1], 0, OP1)
            if i >= LAG:
                stage_b(*seq[i - LAG], ps.pop(i - LAG))
        out_proj(jnp.maximum(t - 1, 0), o_prev[OP1:], OP1, TQ - OP1)

        if not first:
            @pl.when(t >= PLAG)
            def _():
                out_copy(t - PLAG).start()

    def fast_first(t, carry):
        fast_iter(t, True)
        return carry

    def fast_rest(t, carry):
        fast_iter(t, False)
        return carry

    def slow_iter(t, carry):
        g = t % NG
        cols = pl.ds(pl.multiple_of((t // NG) * TQ, TQ), TQ)
        op_v[...] = ot_v[...].T

        def proj(i, c2):
            r0 = pl.multiple_of(i * PR, PR)
            out_proj(jnp.maximum(t - 1, 0), op_v[pl.ds(r0, PR), :], r0, PR)
            return c2
        lax.fori_loop(0, TQ // PR, proj, 0)
        ln2_part(jnp.maximum(t - PLAG, 0))
        row_head = lax.broadcasted_iota(jnp.int32, (128, TQ), 0) // DH

        def head(j, c2):
            qt = qt_v[pl.ds(pl.multiple_of(g * 128, 128), 128), cols]
            w = jnp.where(row_head == j, qt, jnp.zeros_like(qt))
            hrows = pl.ds(pl.multiple_of(g * 128 + j * DH, DH), DH)

            def scores(c, m):
                keys = pl.ds(pl.multiple_of(c * CK, CK), CK)
                s = jnp.dot(k_v[g, keys, :], w, preferred_element_type=F32)
                s_v[keys, :] = s
                return jnp.maximum(m, jnp.max(s.reshape(CK // 8, 8, TQ), axis=0))
            m = lax.fori_loop(0, NC, scores, jnp.full((8, TQ), -jnp.inf, F32))
            m = jnp.max(m, axis=0, keepdims=True)

            def values(c, lo):
                keys = pl.ds(pl.multiple_of(c * CK, CK), CK)
                p = jnp.exp2(s_v[keys, :] - m)
                lc = jnp.sum(p.reshape(CK // 8, 8, TQ), axis=0)
                oc = lax.dot_general(vt_v[hrows, keys], p, NN, preferred_element_type=F32)
                return lo[0] + lc, lo[1] + oc
            l, o = lax.fori_loop(
                0, NC, values, (jnp.zeros((8, TQ), F32), jnp.zeros((DH, TQ), F32)))
            lsum = jnp.sum(l, axis=0, keepdims=True)
            ot_v[pl.ds(pl.multiple_of(j * DH, DH), DH), :] = (o / lsum).astype(BF16)
            return c2
        lax.fori_loop(0, GH, head, 0)

        @pl.when(t >= PLAG)
        def _():
            out_copy(t - PLAG).start()
        return carry

    @pl.when(fast)
    def _():
        lax.fori_loop(0, NG - 1, fast_first, 0)
        lax.fori_loop(NG - 1, NIT, fast_rest, 0)

    @pl.when(jnp.logical_not(fast))
    def _():
        lax.fori_loop(0, NIT, slow_iter, 0)

    wg_copy.wait()
    wu_copy.wait()
    wd_copy.wait()
    for p in range(NIT - PLAG - 1):
        out_copy(p).wait()
    o_last = ot_v[...].T
    for p in range(NIT - PLAG, NP):
        r0 = p * PR - (NQ - 1) * TQ
        if r0 >= 0:
            out_proj(NIT - 1, o_last[r0:r0 + PR], r0, PR)
        ln2_part(p)
    for p in range(NIT - PLAG, NP):
        out_copy(p).start()

    def all_max(v):
        return jnp.max(jnp.max(v, axis=0, keepdims=True), axis=1, keepdims=True)

    def all_min(v):
        return jnp.min(jnp.min(v, axis=0, keepdims=True), axis=1, keepdims=True)

    r = r_v[pl.ds(0, NP), :]
    pos = (lax.broadcasted_iota(jnp.int32, (NP, PR), 0) * PR
           + lax.broadcasted_iota(jnp.int32, (NP, PR), 1))
    m1 = all_max(r)
    p1 = jnp.minimum(all_min(jnp.where(r == m1, pos, S)), S - 1)
    r2 = jnp.where(pos == p1, -jnp.inf, r)
    m2 = all_max(r2)
    p2 = jnp.minimum(all_min(jnp.where(r2 == m2, pos, S)), S - 1)
    i1 = p1[0, 0]
    i2 = p2[0, 0]

    row16 = lax.broadcasted_iota(jnp.int32, (SLAB, D), 0)
    xs = jnp.where(row16 == 0, hn_v[pl.ds(i1, 1), :], hn_v[pl.ds(i2, 1), :]).astype(BF16)
    gate = jnp.dot(xs, wg_v[...], preferred_element_type=F32)
    up = jnp.dot(xs, wu_v[...], preferred_element_type=F32)
    act = (gate * jax.nn.sigmoid(gate) * up).astype(BF16)
    y = jnp.dot(act, wd_v[...], preferred_element_type=F32)
    y = y * jax.nn.sigmoid(jnp.where(row16 == 0, m1, m2))
    y1 = y[0:1]
    y2 = y[1:2]

    for p in range(NIT - PLAG - 1, NP):
        out_copy(p).wait()

    def patch(slot, idx):
        base = pl.multiple_of((idx // SLAB) * SLAB, SLAB)
        rows = pl.ds(base, SLAB)
        rid = row16 + base
        upd = jnp.where(rid == i1, y1, 0.0) + jnp.where(rid == i2, y2, 0.0)
        slab_v[slot] = (h_v[rows, :] + (hn_v[rows, :] + upd)).astype(BF16)
        return pltpu.make_async_copy(slab_v.at[slot], out_hbm.at[rows, :],
                                     patch_sems.at[slot])

    cp1 = patch(0, i1)
    cp1.start()

    @pl.when(i1 // SLAB != i2 // SLAB)
    def _():
        cp2 = patch(1, i2)
        cp2.start()
        cp2.wait()

    cp1.wait()


@jax.jit
def pallas_sequential_preLN__mha_block__moe_arch_mod__prompt_kernel(
    A_x: jax.Array,
    A_wqkv: jax.Array,
    A_wo: jax.Array,
    B_x: jax.Array,
    B_w_r: jax.Array,
    B_w_gate: jax.Array,
    B_w_up: jax.Array,
    B_w_down: jax.Array,
):
    del B_x
    any_spec = pl.BlockSpec(memory_space=pl.ANY)
    out = pl.pallas_call(
        _kernel,
        out_shape=jax.ShapeDtypeStruct((S, D), BF16),
        in_specs=[any_spec] * 7,
        out_specs=any_spec,
        scratch_shapes=[
            pltpu.VMEM((S, D), BF16),
            pltpu.VMEM((D, 3 * D), BF16),
            pltpu.VMEM((D, S), BF16),
            pltpu.VMEM((D, S), BF16),
            pltpu.VMEM((GH, NB, DH, 8, 128), F32),
            pltpu.VMEM((NG, NC, 128, NV, 128), F32),
            pltpu.VMEM((NG, S, 128), BF16),
            pltpu.VMEM((NG, NC * NV, 128), F32),
            pltpu.VMEM((S, D), BF16),
            pltpu.VMEM((2 * D, D), BF16),
            pltpu.VMEM((S, D), F32),
            pltpu.VMEM((D, D), BF16),
            pltpu.VMEM((16 * D,), BF16),
            pltpu.VMEM((128, TQ), BF16),
            pltpu.VMEM((2 * NP, PR), F32),
            pltpu.VMEM((TQ, 128), BF16),
            pltpu.VMEM((2, SLAB, D), BF16),
            pltpu.VMEM((D, F), BF16),
            pltpu.VMEM((D, F), BF16),
            pltpu.VMEM((F, D), BF16),
            pltpu.VMEM((S, TQ), F32),
            pltpu.VMEM((S, D), F32),
            pltpu.VMEM((S, D), BF16),
            pltpu.SemaphoreType.DMA((NXS + 8,)),
            pltpu.SemaphoreType.DMA((NP,)),
            pltpu.SemaphoreType.DMA((2,)),
        ],
        compiler_params=pltpu.CompilerParams(vmem_limit_bytes=120 * 1024 * 1024),
    )(A_x.reshape(S, D), A_wqkv, A_wo, B_w_r, B_w_gate, B_w_up, B_w_down)
    return out.reshape(1, S, D)
```

```python
import math

import jax
import jax.numpy as jnp
from jax import lax
import jax.experimental.pallas as pl
import jax.experimental.pallas.tpu as pltpu

S = 2048
D = 512
H = 32
DH = D // H
F = 1792
EPS = 1e-5
GH = 128 // DH
NG = H // GH
TQ = 512
NQ = S // TQ
NB = TQ // 128
NIT = NQ * NG
CK = 128
NC = S // CK
NV = 16
NM = CK - NV
LAG = 2
XSPLIT = (0, 256, 640, 1152, S)
NXS = len(XSPLIT) - 1
WQV_STEP = 11
PR = 128
NP = S // PR
PLAG = NG + 1
OP1 = 384
SLAB = 16

QSCALE = (DH ** -0.5) * math.log2(math.e)
SCORE_LIMIT = 96.0
V_LIMIT = 2.0 ** 20

F32 = jnp.float32
BF16 = jnp.bfloat16
NN = (((1,), (0,)), ((), ()))
NT = (((1,), (1,)), ((), ()))


def _layernorm(x):
    m = jnp.mean(x, axis=-1, keepdims=True)
    xc = x - m
    v = jnp.mean(xc * xc, axis=-1, keepdims=True)
    return xc * lax.rsqrt(v + EPS)


def _kernel(x_hbm, wqkv_hbm, wo_hbm, wr_hbm, wg_hbm, wu_hbm, wd_hbm, out_hbm,
            x_v, wqkv_v, qt_v, vt_v, qb_v, kb_v, k_v, k32_v, xn_v, wqvt_v, h_v, wo_v,
            wr_v, ot_v, r_v, op_v, slab_v, wg_v, wu_v, wd_v, s_v, hn_v, out_v,
            in_sems, out_sems, patch_sems):
    def x_copy(i):
        rows = pl.ds(XSPLIT[i], XSPLIT[i + 1] - XSPLIT[i])
        return pltpu.make_async_copy(x_hbm.at[rows, :], x_v.at[rows, :], in_sems.at[i])

    def w_copy(part):
        cols = pl.ds(part * D, D)
        return pltpu.make_async_copy(
            wqkv_hbm.at[:, cols], wqkv_v.at[:, cols], in_sems.at[NXS + part])

    wo_copy = pltpu.make_async_copy(wo_hbm, wo_v, in_sems.at[NXS + 3])
    wr_copy = pltpu.make_async_copy(wr_hbm, wr_v.at[pl.ds(0, D)], in_sems.at[NXS + 4])
    wg_copy = pltpu.make_async_copy(wg_hbm, wg_v, in_sems.at[NXS + 5])
    wu_copy = pltpu.make_async_copy(wu_hbm, wu_v, in_sems.at[NXS + 6])
    wd_copy = pltpu.make_async_copy(wd_hbm, wd_v, in_sems.at[NXS + 7])

    x_copy(0).start()
    w_copy(1).start()
    for i in range(1, NXS):
        x_copy(i).start()
    w_copy(0).start()
    w_copy(2).start()
    wo_copy.start()
    wr_copy.start()

    def ln1_step(s):
        rows = pl.ds(s * CK, CK)
        xf = x_v[rows, :].astype(F32)
        h_v[rows, :] = xf
        xn = _layernorm(xf).astype(BF16)
        xn_v[rows, :] = xn
        return xn

    def k_store(s, kk, kabs):
        for g in range(NG):
            k_v[g, pl.ds(s * CK, CK), :] = kk[:, g * 128:(g + 1) * 128].astype(BF16)
            k32_v[g, pl.ds(s * NV, NV), :] = kk[:NV, g * 128:(g + 1) * 128]
        ka = jnp.max(jnp.abs(kk).reshape(CK // 8, 8, D), axis=0)
        return ka if kabs is None else jnp.maximum(kabs, ka)

    ot_v[...] = jnp.zeros_like(ot_v)
    x_copy(0).wait()
    xn = ln1_step(0)
    w_copy(1).wait()
    kabs = None
    kk_prev = None
    for s in range(NC):
        if (s + 1) * CK in XSPLIT[1:-1]:
            x_copy(XSPLIT.index((s + 1) * CK)).wait()
        if s == WQV_STEP:
            w_copy(0).wait()
            w_copy(2).wait()
            wg_copy.start()
            wu_copy.start()
            wd_copy.start()
            wqvt_v[pl.ds(0, D), :] = wqkv_v[:, pl.ds(0, D)].T
            wqvt_v[pl.ds(D, D), :] = wqkv_v[:, pl.ds(2 * D, D)].T
        if kk_prev is not None:
            kabs = k_store(s - 1, kk_prev, kabs)
        xn_next = ln1_step(s + 1) if s + 1 < NC else None
        kk_prev = jnp.dot(xn, wqkv_v[:, pl.ds(D, D)], preferred_element_type=F32)
        xn = xn_next
    kabs = k_store(NC - 1, kk_prev, kabs)

    def qv_block(b, carry):
        vabs, qsum = carry
        rows = pl.ds(pl.multiple_of(b * TQ, TQ), TQ)
        xn = xn_v[rows, :]
        qs = []
        for r0 in range(0, D, 128):
            qt = lax.dot_general(wqvt_v[pl.ds(r0, 128), :], xn, NT,
                                 preferred_element_type=F32) * QSCALE
            qt_v[pl.ds(r0, 128), rows] = qt.astype(BF16)
            qs.append(jnp.sum(jnp.abs(qt).reshape(GH, DH, TQ), axis=1))
        for jj in range(GH // NQ):
            j = b * (GH // NQ) + jj
            q0 = qt_v[pl.ds(pl.multiple_of(j * DH, DH), DH), pl.ds(0, TQ)].astype(F32)
            for cb in range(NB):
                qb_v[j, cb] = jnp.broadcast_to(
                    q0[:, None, cb * 128:(cb + 1) * 128], (DH, 8, 128))
        for r0 in range(0, D, 128):
            vt = lax.dot_general(wqvt_v[pl.ds(D + r0, 128), :], xn, NT,
                                 preferred_element_type=F32)
            vt_v[pl.ds(r0, 128), rows] = vt.astype(BF16)
            vabs = jnp.maximum(vabs, jnp.max(jnp.abs(vt).reshape(16, 8, TQ), axis=0))
        ncb = NC // NQ
        kk = k32_v[0, pl.ds(pl.multiple_of(b * ncb * NV, ncb * NV), ncb * NV), :]
        for d in range(128):
            kb_v[0, pl.ds(b * ncb, ncb), d] = jnp.broadcast_to(
                kk[:, d:d + 1], (ncb * NV, 128)).reshape(ncb, NV, 128)
        return vabs, jnp.maximum(qsum, jnp.concatenate(qs, axis=0))

    vabs, qsum = lax.fori_loop(
        0, NQ, qv_block, (jnp.zeros((8, TQ), F32), jnp.zeros((H, TQ), F32)), unroll=2)

    bound = jnp.max(qsum) * jnp.max(kabs) * 1.02
    fast = jnp.logical_and(bound <= SCORE_LIMIT, jnp.max(vabs) <= V_LIMIT)
    wo_copy.wait()
    wr_copy.wait()

    def out_proj(t, o_rows, r0, nrows):
        rows = pl.ds(pl.multiple_of((t // NG) * TQ + r0, PR), nrows)
        wo_g = wo_v[pl.ds(pl.multiple_of((t % NG) * 128, 128), 128), :]
        h_v[rows, :] = h_v[rows, :] + jnp.dot(o_rows, wo_g, preferred_element_type=F32)

    def ln2_part(p):
        rows = pl.ds(pl.multiple_of(p * PR, PR), PR)
        h = h_v[rows, :]
        hn = _layernorm(h)
        hn_v[rows, :] = hn
        out_v[rows, :] = (h + hn).astype(BF16)
        t = hn * wr_v[pl.ds(0, D)].astype(F32).reshape(1, D)
        t = (t[:, 0:128] + t[:, 128:256]) + (t[:, 256:384] + t[:, 384:512])
        r_v[pl.ds(p, 1), :] = jnp.sum(t.T, axis=0, keepdims=True)

    def out_copy(p):
        rows = pl.ds(pl.multiple_of(p * PR, PR), PR)
        return pltpu.make_async_copy(out_v.at[rows, :], out_hbm.at[rows, :],
                                     out_sems.at[p])

    def head_weights(g, j, cols):
        q = qt_v[pl.ds(pl.multiple_of(g * 128 + j * DH, DH), DH), cols]
        parts = []
        if j > 0:
            parts.append(jnp.zeros((j * DH, TQ), BF16))
        parts.append(q)
        if j < GH - 1:
            parts.append(jnp.zeros(((GH - 1 - j) * DH, TQ), BF16))
        return jnp.concatenate(parts, axis=0)

    def vpu_scores(kb, j, c):
        keys = kb[0, c, pl.ds(j * DH, DH)].reshape(DH, NV // 8, 8, 128)
        res = []
        prev = None
        for b in range(NB):
            terms = keys * qb_v[j, b][:, None]
            cur = prev
            for d in range(DH):
                cur = terms[d] if cur is None else cur + terms[d]
            res.append(cur if prev is None else cur - prev)
            prev = cur
        return jnp.concatenate(res, axis=2).reshape(NV, TQ)

    def fast_iter(t, first):
        g = t % NG
        cols = pl.ds(pl.multiple_of((t // NG) * TQ, TQ), TQ)
        o_prev = ot_v[...].T
        if first:
            kb = kb_v.at[pl.ds(g, 2)]
            kk = k32_v[g + 1]
            for d in range(128):
                kb[1, :, d] = jnp.broadcast_to(
                    kk[:, d:d + 1], (NC * NV, 128)).reshape(NC, NV, 128)
        else:
            kb = kb_v.at[pl.ds(g, 1)]
            ln2_part(jnp.maximum(t - PLAG, 0))
        st = {}

        def q_refill(j, c, tie):
            if c % 2:
                return
            js = (j - 1) % GH
            tn = t if j == 0 else jnp.minimum(t + 1, NIT - 1)
            b, d0 = c // 4, (c % 4) * 4
            qn = qt_v[pl.ds(pl.multiple_of((tn % NG) * 128 + js * DH, DH), DH),
                      pl.ds(pl.multiple_of((tn // NG) * TQ + b * 128, 128), 128)]
            qn = qn.astype(F32)[d0:d0 + 8] + tie * 0.0
            qb_v[js, b, pl.ds(d0, 8)] = jnp.broadcast_to(qn[:, None, :], (8, 8, 128))

        def stage_a(j, c):
            if c == 0:
                st[j] = dict(w=head_weights(g, j, cols))
            s = jnp.dot(k_v[g, pl.ds(c * CK + NV, NM), :], st[j]['w'],
                        preferred_element_type=F32)
            p = jnp.exp2(s)
            lc = jnp.sum(p.reshape(NM // 8, 8, TQ), axis=0)
            pv = jnp.exp2(vpu_scores(kb, j, c))
            lc = lc + jnp.sum(pv.reshape(NV // 8, 8, TQ), axis=0)
            st[j]['l'] = lc if c == 0 else lc + st[j]['l']
            return jnp.concatenate([pv, p], axis=0)

        def stage_b(j, c, p):
            hrows = pl.ds(pl.multiple_of(g * 128 + j * DH, DH), DH)
            vt = vt_v[hrows, pl.ds(c * CK, CK)]
            if first:
                oc = jnp.concatenate(
                    [lax.dot_general(vt, p[:, :128].astype(BF16), NN,
                                     preferred_element_type=F32),
                     lax.dot_general(vt, p[:, 128:], NN, preferred_element_type=F32)],
                    axis=1)
            else:
                oc = lax.dot_general(vt, p, NN, preferred_element_type=F32)
            q_refill(j, c, oc[:8, :128])
            st[j]['o'] = oc if c == 0 else oc + st[j]['o']
            if c == NC - 1:
                lsum = jnp.sum(st[j]['l'], axis=0, keepdims=True)
                ot_v[pl.ds(j * DH, DH), :] = (st[j]['o'] / lsum).astype(BF16)

        seq = [(j, c) for j in range(GH) for c in range(NC)]
        ps = {}
        for i in range(len(seq) + LAG):
            if i < len(seq):
                ps[i] = stage_a(*seq[i])
            if i == len(seq):
                out_proj(jnp.maximum(t - 1, 0), o_prev[:OP1], 0, OP1)
            if i >= LAG:
                stage_b(*seq[i - LAG], ps.pop(i - LAG))
        out_proj(jnp.maximum(t - 1, 0), o_prev[OP1:], OP1, TQ - OP1)

        if not first:
            @pl.when(t >= PLAG)
            def _():
                out_copy(t - PLAG).start()

    def fast_first(t, carry):
        fast_iter(t, True)
        return carry

    def fast_rest(t, carry):
        fast_iter(t, False)
        return carry

    def slow_iter(t, carry):
        g = t % NG
        cols = pl.ds(pl.multiple_of((t // NG) * TQ, TQ), TQ)
        op_v[...] = ot_v[...].T

        def proj(i, c2):
            r0 = pl.multiple_of(i * PR, PR)
            out_proj(jnp.maximum(t - 1, 0), op_v[pl.ds(r0, PR), :], r0, PR)
            return c2
        lax.fori_loop(0, TQ // PR, proj, 0)
        ln2_part(jnp.maximum(t - PLAG, 0))
        row_head = lax.broadcasted_iota(jnp.int32, (128, TQ), 0) // DH

        def head(j, c2):
            qt = qt_v[pl.ds(pl.multiple_of(g * 128, 128), 128), cols]
            w = jnp.where(row_head == j, qt, jnp.zeros_like(qt))
            hrows = pl.ds(pl.multiple_of(g * 128 + j * DH, DH), DH)

            def scores(c, m):
                keys = pl.ds(pl.multiple_of(c * CK, CK), CK)
                s = jnp.dot(k_v[g, keys, :], w, preferred_element_type=F32)
                s_v[keys, :] = s
                return jnp.maximum(m, jnp.max(s.reshape(CK // 8, 8, TQ), axis=0))
            m = lax.fori_loop(0, NC, scores, jnp.full((8, TQ), -jnp.inf, F32))
            m = jnp.max(m, axis=0, keepdims=True)

            def values(c, lo):
                keys = pl.ds(pl.multiple_of(c * CK, CK), CK)
                p = jnp.exp2(s_v[keys, :] - m)
                lc = jnp.sum(p.reshape(CK // 8, 8, TQ), axis=0)
                oc = lax.dot_general(vt_v[hrows, keys], p, NN, preferred_element_type=F32)
                return lo[0] + lc, lo[1] + oc
            l, o = lax.fori_loop(
                0, NC, values, (jnp.zeros((8, TQ), F32), jnp.zeros((DH, TQ), F32)))
            lsum = jnp.sum(l, axis=0, keepdims=True)
            ot_v[pl.ds(pl.multiple_of(j * DH, DH), DH), :] = (o / lsum).astype(BF16)
            return c2
        lax.fori_loop(0, GH, head, 0)

        @pl.when(t >= PLAG)
        def _():
            out_copy(t - PLAG).start()
        return carry

    @pl.when(fast)
    def _():
        lax.fori_loop(0, NG - 1, fast_first, 0)
        lax.fori_loop(NG - 1, NIT, fast_rest, 0)

    @pl.when(jnp.logical_not(fast))
    def _():
        lax.fori_loop(0, NIT, slow_iter, 0)

    wg_copy.wait()
    wu_copy.wait()
    wd_copy.wait()
    for p in range(NIT - PLAG - 1):
        out_copy(p).wait()
    o_last = ot_v[...].T
    for p in range(NIT - PLAG, NP):
        r0 = p * PR - (NQ - 1) * TQ
        if r0 >= 0:
            out_proj(NIT - 1, o_last[r0:r0 + PR], r0, PR)
        ln2_part(p)
    for p in range(NIT - PLAG, NP):
        out_copy(p).start()

    def all_max(v):
        return jnp.max(jnp.max(v, axis=0, keepdims=True), axis=1, keepdims=True)

    def all_min(v):
        return jnp.min(jnp.min(v, axis=0, keepdims=True), axis=1, keepdims=True)

    r = r_v[pl.ds(0, NP), :]
    pos = (lax.broadcasted_iota(jnp.int32, (NP, PR), 0) * PR
           + lax.broadcasted_iota(jnp.int32, (NP, PR), 1))
    m1 = all_max(r)
    p1 = jnp.minimum(all_min(jnp.where(r == m1, pos, S)), S - 1)
    r2 = jnp.where(pos == p1, -jnp.inf, r)
    m2 = all_max(r2)
    p2 = jnp.minimum(all_min(jnp.where(r2 == m2, pos, S)), S - 1)
    i1 = p1[0, 0]
    i2 = p2[0, 0]

    row16 = lax.broadcasted_iota(jnp.int32, (SLAB, D), 0)
    xs = jnp.where(row16 == 0, hn_v[pl.ds(i1, 1), :], hn_v[pl.ds(i2, 1), :]).astype(BF16)
    gate = jnp.dot(xs, wg_v[...], preferred_element_type=F32)
    up = jnp.dot(xs, wu_v[...], preferred_element_type=F32)
    act = (gate * jax.nn.sigmoid(gate) * up).astype(BF16)
    y = jnp.dot(act, wd_v[...], preferred_element_type=F32)
    y = y * jax.nn.sigmoid(jnp.where(row16 == 0, m1, m2))
    y1 = y[0:1]
    y2 = y[1:2]

    for p in range(NIT - PLAG - 1, NP):
        out_copy(p).wait()

    def patch(slot, idx):
        base = pl.multiple_of((idx // SLAB) * SLAB, SLAB)
        rows = pl.ds(base, SLAB)
        rid = row16 + base
        upd = jnp.where(rid == i1, y1, 0.0) + jnp.where(rid == i2, y2, 0.0)
        slab_v[slot] = (h_v[rows, :] + (hn_v[rows, :] + upd)).astype(BF16)
        return pltpu.make_async_copy(slab_v.at[slot], out_hbm.at[rows, :],
                                     patch_sems.at[slot])

    cp1 = patch(0, i1)
    cp1.start()

    @pl.when(i1 // SLAB != i2 // SLAB)
    def _():
        cp2 = patch(1, i2)
        cp2.start()
        cp2.wait()

    cp1.wait()


@jax.jit
def pallas_sequential_preLN__mha_block__moe_arch_mod__prompt_kernel(
    A_x: jax.Array,
    A_wqkv: jax.Array,
    A_wo: jax.Array,
    B_x: jax.Array,
    B_w_r: jax.Array,
    B_w_gate: jax.Array,
    B_w_up: jax.Array,
    B_w_down: jax.Array,
):
    del B_x
    any_spec = pl.BlockSpec(memory_space=pl.ANY)
    out = pl.pallas_call(
        _kernel,
        out_shape=jax.ShapeDtypeStruct((S, D), BF16),
        in_specs=[any_spec] * 7,
        out_specs=any_spec,
        scratch_shapes=[
            pltpu.VMEM((S, D), BF16),
            pltpu.VMEM((D, 3 * D), BF16),
            pltpu.VMEM((D, S), BF16),
            pltpu.VMEM((D, S), BF16),
            pltpu.VMEM((GH, NB, DH, 8, 128), F32),
            pltpu.VMEM((NG, NC, 128, NV, 128), F32),
            pltpu.VMEM((NG, S, 128), BF16),
            pltpu.VMEM((NG, NC * NV, 128), F32),
            pltpu.VMEM((S, D), BF16),
            pltpu.VMEM((2 * D, D), BF16),
            pltpu.VMEM((S, D), F32),
            pltpu.VMEM((D, D), BF16),
            pltpu.VMEM((16 * D,), BF16),
            pltpu.VMEM((128, TQ), BF16),
            pltpu.VMEM((2 * NP, PR), F32),
            pltpu.VMEM((TQ, 128), BF16),
            pltpu.VMEM((2, SLAB, D), BF16),
            pltpu.VMEM((D, F), BF16),
            pltpu.VMEM((D, F), BF16),
            pltpu.VMEM((F, D), BF16),
            pltpu.VMEM((S, TQ), F32),
            pltpu.VMEM((S, D), F32),
            pltpu.VMEM((S, D), BF16),
            pltpu.SemaphoreType.DMA((NXS + 8,)),
            pltpu.SemaphoreType.DMA((NP,)),
            pltpu.SemaphoreType.DMA((2,)),
        ],
        compiler_params=pltpu.CompilerParams(vmem_limit_bytes=120 * 1024 * 1024),
    )(A_x.reshape(S, D), A_wqkv, A_wo, B_w_r, B_w_gate, B_w_up, B_w_down)
    return out.reshape(1, S, D)
```

```python
import math

import jax
import jax.numpy as jnp
from jax import lax
import jax.experimental.pallas as pl
import jax.experimental.pallas.tpu as pltpu

S = 2048
D = 512
H = 32
DH = D // H
F = 1792
EPS = 1e-5
GH = 128 // DH
NG = H // GH
TQ = 512
NQ = S // TQ
NB = TQ // 128
NIT = NQ * NG
CK = 128
NC = S // CK
NV = 16
NM = CK - NV
LAG = 2
XSPLIT = (0, 256, 640, 1152, S)
NXS = len(XSPLIT) - 1
WQV_STEP = 11
PR = 128
NP = S // PR
PLAG = NG + 1
OP1 = 384
KPRE = 2
SLAB = 16

QSCALE = (DH ** -0.5) * math.log2(math.e)
SCORE_LIMIT = 96.0
V_LIMIT = 2.0 ** 16

F32 = jnp.float32
BF16 = jnp.bfloat16
NN = (((1,), (0,)), ((), ()))
NT = (((1,), (1,)), ((), ()))


def _layernorm(x):
    m = jnp.mean(x, axis=-1, keepdims=True)
    xc = x - m
    v = jnp.mean(xc * xc, axis=-1, keepdims=True)
    return xc * lax.rsqrt(v + EPS)


def _kernel(x_hbm, wqkv_hbm, wo_hbm, wr_hbm, wg_hbm, wu_hbm, wd_hbm, out_hbm,
            x_v, wqkv_v, qt_v, vt_v, qb_v, kb_v, k_v, k32_v, xn_v, wqvt_v, h_v, wo_v,
            wr_v, ot_v, r_v, op_v, slab_v, wg_v, wu_v, wd_v, s_v, hn_v, out_v,
            in_sems, out_sems, patch_sems):
    def x_copy(i):
        rows = pl.ds(XSPLIT[i], XSPLIT[i + 1] - XSPLIT[i])
        return pltpu.make_async_copy(x_hbm.at[rows, :], x_v.at[rows, :], in_sems.at[i])

    def w_copy(part):
        cols = pl.ds(part * D, D)
        return pltpu.make_async_copy(
            wqkv_hbm.at[:, cols], wqkv_v.at[:, cols], in_sems.at[NXS + part])

    wo_copy = pltpu.make_async_copy(wo_hbm, wo_v, in_sems.at[NXS + 3])
    wr_copy = pltpu.make_async_copy(wr_hbm, wr_v.at[pl.ds(0, D)], in_sems.at[NXS + 4])
    wg_copy = pltpu.make_async_copy(wg_hbm, wg_v, in_sems.at[NXS + 5])
    wu_copy = pltpu.make_async_copy(wu_hbm, wu_v, in_sems.at[NXS + 6])
    wd_copy = pltpu.make_async_copy(wd_hbm, wd_v, in_sems.at[NXS + 7])

    x_copy(0).start()
    w_copy(1).start()
    for i in range(1, NXS):
        x_copy(i).start()
    w_copy(0).start()
    w_copy(2).start()
    wo_copy.start()
    wr_copy.start()

    def ln1_step(s):
        rows = pl.ds(s * CK, CK)
        xf = x_v[rows, :].astype(F32)
        h_v[rows, :] = xf
        xn = _layernorm(xf).astype(BF16)
        xn_v[rows, :] = xn
        return xn

    def k_store(s, kk, kabs):
        for g in range(NG):
            k_v[g, pl.ds(s * CK, CK), :] = kk[:, g * 128:(g + 1) * 128].astype(BF16)
            if g >= KPRE:
                k32_v[g - KPRE, pl.ds(s * NV, NV), :] = kk[:NV, g * 128:(g + 1) * 128]
        ka = jnp.max(jnp.abs(kk).reshape(CK // 8, 8, D), axis=0)
        return ka if kabs is None else jnp.maximum(kabs, ka)

    ot_v[...] = jnp.zeros_like(ot_v)
    x_copy(0).wait()
    xn = ln1_step(0)
    w_copy(1).wait()
    kabs = None
    kk_prev = None
    for s in range(NC):
        if (s + 1) * CK in XSPLIT[1:-1]:
            x_copy(XSPLIT.index((s + 1) * CK)).wait()
        if s == WQV_STEP:
            w_copy(0).wait()
            w_copy(2).wait()
            wg_copy.start()
            wu_copy.start()
            wd_copy.start()
            wqvt_v[pl.ds(0, D), :] = wqkv_v[:, pl.ds(0, D)].T
            wqvt_v[pl.ds(D, D), :] = wqkv_v[:, pl.ds(2 * D, D)].T
        if kk_prev is not None:
            kabs = k_store(s - 1, kk_prev, kabs)
        xn_next = ln1_step(s + 1) if s + 1 < NC else None
        kk_prev = jnp.dot(xn, wqkv_v[:, pl.ds(D, D)], preferred_element_type=F32)
        xn = xn_next
    kabs = k_store(NC - 1, kk_prev, kabs)

    def qv_block(b, carry):
        vabs, qsum = carry
        rows = pl.ds(pl.multiple_of(b * TQ, TQ), TQ)
        xn = xn_v[rows, :]
        qs = []
        for r0 in range(0, D, 128):
            qt = lax.dot_general(wqvt_v[pl.ds(r0, 128), :], xn, NT,
                                 preferred_element_type=F32) * QSCALE
            qt_v[pl.ds(r0, 128), rows] = qt.astype(BF16)
            qs.append(jnp.sum(jnp.abs(qt).reshape(GH, DH, TQ), axis=1))
        for jj in range(GH // NQ):
            j = b * (GH // NQ) + jj
            q0 = qt_v[pl.ds(pl.multiple_of(j * DH, DH), DH), pl.ds(0, TQ)].astype(F32)
            for cb in range(NB):
                qb_v[j, cb] = jnp.broadcast_to(
                    q0[:, None, cb * 128:(cb + 1) * 128], (DH, 8, 128))
        for r0 in range(0, D, 128):
            vt = lax.dot_general(wqvt_v[pl.ds(D + r0, 128), :], xn, NT,
                                 preferred_element_type=F32)
            vt_v[pl.ds(r0, 128), rows] = vt.astype(BF16)
            vabs = jnp.maximum(vabs, jnp.max(jnp.abs(vt).reshape(16, 8, TQ), axis=0))
        ncb = NC // NQ
        for g in range(KPRE):
            kk = jnp.concatenate(
                [k_v[g, pl.ds(pl.multiple_of((b * ncb + c) * CK, CK), NV), :]
                 for c in range(ncb)], axis=0).astype(F32)
            for d in range(128):
                kb_v[g, pl.ds(b * ncb, ncb), d] = jnp.broadcast_to(
                    kk[:, d:d + 1], (ncb * NV, 128)).reshape(ncb, NV, 128)
        return vabs, jnp.maximum(qsum, jnp.concatenate(qs, axis=0))

    vabs, qsum = lax.fori_loop(
        0, NQ, qv_block, (jnp.zeros((8, TQ), F32), jnp.zeros((H, TQ), F32)), unroll=2)

    bound = jnp.max(qsum) * jnp.max(kabs) * 1.02
    fast = jnp.logical_and(bound <= SCORE_LIMIT, jnp.max(vabs) <= V_LIMIT)
    wo_copy.wait()
    wr_copy.wait()

    def out_proj(t, o_rows, r0, nrows):
        rows = pl.ds(pl.multiple_of((t // NG) * TQ + r0, PR), nrows)
        wo_g = wo_v[pl.ds(pl.multiple_of((t % NG) * 128, 128), 128), :]
        h_v[rows, :] = h_v[rows, :] + jnp.dot(o_rows, wo_g, preferred_element_type=F32)

    def ln2_part(p):
        rows = pl.ds(pl.multiple_of(p * PR, PR), PR)
        h = h_v[rows, :]
        hn = _layernorm(h)
        hn_v[rows, :] = hn
        out_v[rows, :] = (h + hn).astype(BF16)
        t = hn * wr_v[pl.ds(0, D)].astype(F32).reshape(1, D)
        t = (t[:, 0:128] + t[:, 128:256]) + (t[:, 256:384] + t[:, 384:512])
        r_v[pl.ds(p, 1), :] = jnp.sum(t.T, axis=0, keepdims=True)

    def out_copy(p):
        rows = pl.ds(pl.multiple_of(p * PR, PR), PR)
        return pltpu.make_async_copy(out_v.at[rows, :], out_hbm.at[rows, :],
                                     out_sems.at[p])

    def head_weights(g, j, cols):
        q = qt_v[pl.ds(pl.multiple_of(g * 128 + j * DH, DH), DH), cols]
        parts = []
        if j > 0:
            parts.append(jnp.zeros((j * DH, TQ), BF16))
        parts.append(q)
        if j < GH - 1:
            parts.append(jnp.zeros(((GH - 1 - j) * DH, TQ), BF16))
        return jnp.concatenate(parts, axis=0)

    def vpu_scores(kb, j, c):
        keys = kb[0, c, pl.ds(j * DH, DH)].reshape(DH, NV // 8, 8, 128)
        res = []
        prev = None
        for b in range(NB):
            terms = keys * qb_v[j, b][:, None]
            cur = prev
            for d in range(DH):
                cur = terms[d] if cur is None else cur + terms[d]
            res.append(cur if prev is None else cur - prev)
            prev = cur
        return jnp.concatenate(res, axis=2).reshape(NV, TQ)

    def fast_iter(t, first):
        g = t % NG
        cols = pl.ds(pl.multiple_of((t // NG) * TQ, TQ), TQ)
        o_prev = ot_v[...].T
        if first:
            kb = kb_v.at[pl.ds(g, KPRE + 1)]
            kk = k32_v[g]
            for d in range(128):
                kb[KPRE, :, d] = jnp.broadcast_to(
                    kk[:, d:d + 1], (NC * NV, 128)).reshape(NC, NV, 128)
        else:
            kb = kb_v.at[pl.ds(g, 1)]
            ln2_part(jnp.maximum(t - PLAG, 0))
        st = {}

        def q_refill(j, c, tie):
            if c % 2:
                return
            js = (j - 1) % GH
            tn = t if j == 0 else jnp.minimum(t + 1, NIT - 1)
            b, d0 = c // 4, (c % 4) * 4
            qn = qt_v[pl.ds(pl.multiple_of((tn % NG) * 128 + js * DH, DH), DH),
                      pl.ds(pl.multiple_of((tn // NG) * TQ + b * 128, 128), 128)]
            qn = qn.astype(F32)[d0:d0 + 8] + tie * 0.0
            qb_v[js, b, pl.ds(d0, 8)] = jnp.broadcast_to(qn[:, None, :], (8, 8, 128))

        def stage_a(j, c):
            if c == 0:
                st[j] = dict(w=head_weights(g, j, cols))
            s = jnp.dot(k_v[g, pl.ds(c * CK + NV, NM), :], st[j]['w'],
                        preferred_element_type=F32)
            p = jnp.exp2(s)
            lc = jnp.sum(p.reshape(NM // 8, 8, TQ), axis=0)
            pv = jnp.exp2(vpu_scores(kb, j, c))
            lc = lc + jnp.sum(pv.reshape(NV // 8, 8, TQ), axis=0)
            st[j]['l'] = lc if c == 0 else lc + st[j]['l']
            return jnp.concatenate([pv, p], axis=0)

        def stage_b(j, c, p):
            hrows = pl.ds(pl.multiple_of(g * 128 + j * DH, DH), DH)
            vt = vt_v[hrows, pl.ds(c * CK, CK)]
            if first:
                oc = jnp.concatenate(
                    [lax.dot_general(vt, p[:, :128].astype(BF16), NN,
                                     preferred_element_type=F32),
                     lax.dot_general(vt, p[:, 128:], NN, preferred_element_type=F32)],
                    axis=1)
            else:
                oc = lax.dot_general(vt, p, NN, preferred_element_type=F32)
            q_refill(j, c, oc[:8, :128])
            st[j]['o'] = oc if c == 0 else oc + st[j]['o']
            if c == NC - 1:
                lsum = jnp.sum(st[j]['l'], axis=0, keepdims=True)
                ot_v[pl.ds(j * DH, DH), :] = (st[j]['o'] / lsum).astype(BF16)

        seq = [(j, c) for j in range(GH) for c in range(NC)]
        ps = {}
        for i in range(len(seq) + LAG):
            if i < len(seq):
                ps[i] = stage_a(*seq[i])
            if i == len(seq):
                out_proj(jnp.maximum(t - 1, 0), o_prev[:OP1], 0, OP1)
            if i >= LAG:
                stage_b(*seq[i - LAG], ps.pop(i - LAG))
        out_proj(jnp.maximum(t - 1, 0), o_prev[OP1:], OP1, TQ - OP1)

        if not first:
            @pl.when(t >= PLAG)
            def _():
                out_copy(t - PLAG).start()

    def fast_first(t, carry):
        fast_iter(t, True)
        return carry

    def fast_rest(t, carry):
        fast_iter(t, False)
        return carry

    def slow_iter(t, carry):
        g = t % NG
        cols = pl.ds(pl.multiple_of((t // NG) * TQ, TQ), TQ)
        op_v[...] = ot_v[...].T

        def proj(i, c2):
            r0 = pl.multiple_of(i * PR, PR)
            out_proj(jnp.maximum(t - 1, 0), op_v[pl.ds(r0, PR), :], r0, PR)
            return c2
        lax.fori_loop(0, TQ // PR, proj, 0)
        ln2_part(jnp.maximum(t - PLAG, 0))
        row_head = lax.broadcasted_iota(jnp.int32, (128, TQ), 0) // DH

        def head(j, c2):
            qt = qt_v[pl.ds(pl.multiple_of(g * 128, 128), 128), cols]
            w = jnp.where(row_head == j, qt, jnp.zeros_like(qt))
            hrows = pl.ds(pl.multiple_of(g * 128 + j * DH, DH), DH)

            def scores(c, m):
                keys = pl.ds(pl.multiple_of(c * CK, CK), CK)
                s = jnp.dot(k_v[g, keys, :], w, preferred_element_type=F32)
                s_v[keys, :] = s
                return jnp.maximum(m, jnp.max(s.reshape(CK // 8, 8, TQ), axis=0))
            m = lax.fori_loop(0, NC, scores, jnp.full((8, TQ), -jnp.inf, F32))
            m = jnp.max(m, axis=0, keepdims=True)

            def values(c, lo):
                keys = pl.ds(pl.multiple_of(c * CK, CK), CK)
                p = jnp.exp2(s_v[keys, :] - m)
                lc = jnp.sum(p.reshape(CK // 8, 8, TQ), axis=0)
                oc = lax.dot_general(vt_v[hrows, keys], p, NN, preferred_element_type=F32)
                return lo[0] + lc, lo[1] + oc
            l, o = lax.fori_loop(
                0, NC, values, (jnp.zeros((8, TQ), F32), jnp.zeros((DH, TQ), F32)))
            lsum = jnp.sum(l, axis=0, keepdims=True)
            ot_v[pl.ds(pl.multiple_of(j * DH, DH), DH), :] = (o / lsum).astype(BF16)
            return c2
        lax.fori_loop(0, GH, head, 0)

        @pl.when(t >= PLAG)
        def _():
            out_copy(t - PLAG).start()
        return carry

    @pl.when(fast)
    def _():
        lax.fori_loop(0, NG - KPRE, fast_first, 0)
        lax.fori_loop(NG - KPRE, NIT, fast_rest, 0)

    @pl.when(jnp.logical_not(fast))
    def _():
        lax.fori_loop(0, NIT, slow_iter, 0)

    wg_copy.wait()
    wu_copy.wait()
    wd_copy.wait()
    for p in range(NIT - PLAG - 1):
        out_copy(p).wait()
    o_last = ot_v[...].T
    for p in range(NIT - PLAG, NP):
        r0 = p * PR - (NQ - 1) * TQ
        if r0 >= 0:
            out_proj(NIT - 1, o_last[r0:r0 + PR], r0, PR)
        ln2_part(p)
    for p in range(NIT - PLAG, NP):
        out_copy(p).start()

    def all_max(v):
        return jnp.max(jnp.max(v, axis=0, keepdims=True), axis=1, keepdims=True)

    def all_min(v):
        return jnp.min(jnp.min(v, axis=0, keepdims=True), axis=1, keepdims=True)

    r = r_v[pl.ds(0, NP), :]
    pos = (lax.broadcasted_iota(jnp.int32, (NP, PR), 0) * PR
           + lax.broadcasted_iota(jnp.int32, (NP, PR), 1))
    m1 = all_max(r)
    p1 = jnp.minimum(all_min(jnp.where(r == m1, pos, S)), S - 1)
    r2 = jnp.where(pos == p1, -jnp.inf, r)
    m2 = all_max(r2)
    p2 = jnp.minimum(all_min(jnp.where(r2 == m2, pos, S)), S - 1)
    i1 = p1[0, 0]
    i2 = p2[0, 0]

    row16 = lax.broadcasted_iota(jnp.int32, (SLAB, D), 0)
    xs = jnp.where(row16 == 0, hn_v[pl.ds(i1, 1), :], hn_v[pl.ds(i2, 1), :]).astype(BF16)
    gate = jnp.dot(xs, wg_v[...], preferred_element_type=F32)
    up = jnp.dot(xs, wu_v[...], preferred_element_type=F32)
    act = (gate * jax.nn.sigmoid(gate) * up).astype(BF16)
    y = jnp.dot(act, wd_v[...], preferred_element_type=F32)
    y = y * jax.nn.sigmoid(jnp.where(row16 == 0, m1, m2))
    y1 = y[0:1]
    y2 = y[1:2]

    for p in range(NIT - PLAG - 1, NP):
        out_copy(p).wait()

    def patch(slot, idx):
        base = pl.multiple_of((idx // SLAB) * SLAB, SLAB)
        rows = pl.ds(base, SLAB)
        rid = row16 + base
        upd = jnp.where(rid == i1, y1, 0.0) + jnp.where(rid == i2, y2, 0.0)
        slab_v[slot] = (h_v[rows, :] + (hn_v[rows, :] + upd)).astype(BF16)
        return pltpu.make_async_copy(slab_v.at[slot], out_hbm.at[rows, :],
                                     patch_sems.at[slot])

    cp1 = patch(0, i1)
    cp1.start()

    @pl.when(i1 // SLAB != i2 // SLAB)
    def _():
        cp2 = patch(1, i2)
        cp2.start()
        cp2.wait()

    cp1.wait()


@jax.jit
def pallas_sequential_preLN__mha_block__moe_arch_mod__prompt_kernel(
    A_x: jax.Array,
    A_wqkv: jax.Array,
    A_wo: jax.Array,
    B_x: jax.Array,
    B_w_r: jax.Array,
    B_w_gate: jax.Array,
    B_w_up: jax.Array,
    B_w_down: jax.Array,
):
    del B_x
    any_spec = pl.BlockSpec(memory_space=pl.ANY)
    out = pl.pallas_call(
        _kernel,
        out_shape=jax.ShapeDtypeStruct((S, D), BF16),
        in_specs=[any_spec] * 7,
        out_specs=any_spec,
        scratch_shapes=[
            pltpu.VMEM((S, D), BF16),
            pltpu.VMEM((D, 3 * D), BF16),
            pltpu.VMEM((D, S), BF16),
            pltpu.VMEM((D, S), BF16),
            pltpu.VMEM((GH, NB, DH, 8, 128), F32),
            pltpu.VMEM((NG, NC, 128, NV, 128), F32),
            pltpu.VMEM((NG, S, 128), BF16),
            pltpu.VMEM((NG - KPRE, NC * NV, 128), F32),
            pltpu.VMEM((S, D), BF16),
            pltpu.VMEM((2 * D, D), BF16),
            pltpu.VMEM((S, D), F32),
            pltpu.VMEM((D, D), BF16),
            pltpu.VMEM((16 * D,), BF16),
            pltpu.VMEM((128, TQ), BF16),
            pltpu.VMEM((2 * NP, PR), F32),
            pltpu.VMEM((TQ, 128), BF16),
            pltpu.VMEM((2, SLAB, D), BF16),
            pltpu.VMEM((D, F), BF16),
            pltpu.VMEM((D, F), BF16),
            pltpu.VMEM((F, D), BF16),
            pltpu.VMEM((S, TQ), F32),
            pltpu.VMEM((S, D), F32),
            pltpu.VMEM((S, D), BF16),
            pltpu.SemaphoreType.DMA((NXS + 8,)),
            pltpu.SemaphoreType.DMA((NP,)),
            pltpu.SemaphoreType.DMA((2,)),
        ],
        compiler_params=pltpu.CompilerParams(vmem_limit_bytes=120 * 1024 * 1024),
    )(A_x.reshape(S, D), A_wqkv, A_wo, B_w_r, B_w_gate, B_w_up, B_w_down)
    return out.reshape(1, S, D)
```

```python
import math

import jax
import jax.numpy as jnp
from jax import lax
import jax.experimental.pallas as pl
import jax.experimental.pallas.tpu as pltpu

S = 2048
D = 512
H = 32
DH = D // H
F = 1792
EPS = 1e-5
GH = 128 // DH
NG = H // GH
TQ = 512
NQ = S // TQ
NB = TQ // 128
NIT = NQ * NG
CK = 128
NC = S // CK
NV = 16
NM = CK - NV
LAG = 2
XSPLIT = (0, 256, 640, 1408, S)
NXS = len(XSPLIT) - 1
WQV_STEP = 10
PR = 128
NP = S // PR
PLAG = NG + 1
OP1 = 384
KPRE = 2
SLAB = 16

QSCALE = (DH ** -0.5) * math.log2(math.e)
SCORE_LIMIT = 96.0
V_LIMIT = 2.0 ** 16

F32 = jnp.float32
BF16 = jnp.bfloat16
NN = (((1,), (0,)), ((), ()))
NT = (((1,), (1,)), ((), ()))


def _layernorm(x):
    m = jnp.mean(x, axis=-1, keepdims=True)
    xc = x - m
    v = jnp.mean(xc * xc, axis=-1, keepdims=True)
    return xc * lax.rsqrt(v + EPS)


def _lane_replicate(kk, d0, nblk):
    return jnp.stack(
        [jnp.broadcast_to(kk[:, d:d + 1], (nblk * NV, 128)).reshape(nblk, NV, 128)
         for d in range(d0, d0 + DH)], axis=1)


def _kernel(x_hbm, wqkv_hbm, wo_hbm, wr_hbm, wg_hbm, wu_hbm, wd_hbm, out_hbm,
            x_v, wqkv_v, qt_v, vt_v, qb_v, kb_v, k_v, k32_v, xn_v, wqvt_v, h_v, wo_v,
            wr_v, ot_v, r_v, op_v, slab_v, wg_v, wu_v, wd_v, s_v, hn_v, out_v,
            in_sems, out_sems, patch_sems):
    def x_copy(i):
        rows = pl.ds(XSPLIT[i], XSPLIT[i + 1] - XSPLIT[i])
        return pltpu.make_async_copy(x_hbm.at[rows, :], x_v.at[rows, :], in_sems.at[i])

    def w_copy(part):
        cols = pl.ds(part * D, D)
        return pltpu.make_async_copy(
            wqkv_hbm.at[:, cols], wqkv_v.at[:, cols], in_sems.at[NXS + part])

    wo_copy = pltpu.make_async_copy(wo_hbm, wo_v, in_sems.at[NXS + 3])
    wr_copy = pltpu.make_async_copy(wr_hbm, wr_v.at[pl.ds(0, D)], in_sems.at[NXS + 4])
    wg_copy = pltpu.make_async_copy(wg_hbm, wg_v, in_sems.at[NXS + 5])
    wu_copy = pltpu.make_async_copy(wu_hbm, wu_v, in_sems.at[NXS + 6])
    wd_copy = pltpu.make_async_copy(wd_hbm, wd_v, in_sems.at[NXS + 7])

    x_copy(0).start()
    w_copy(1).start()
    for i in range(1, NXS - 1):
        x_copy(i).start()
    w_copy(0).start()
    w_copy(2).start()
    x_copy(NXS - 1).start()
    wo_copy.start()
    wr_copy.start()

    def ln1_step(s):
        rows = pl.ds(s * CK, CK)
        xf = x_v[rows, :].astype(F32)
        h_v[rows, :] = xf
        xn = _layernorm(xf).astype(BF16)
        xn_v[rows, :] = xn
        return xn

    def k_store(s, kk, kabs):
        for g in range(NG):
            k_v[g, pl.ds(s * CK, CK), :] = kk[:, g * 128:(g + 1) * 128].astype(BF16)
            if g >= KPRE:
                k32_v[g - KPRE, pl.ds(s * NV, NV), :] = kk[:NV, g * 128:(g + 1) * 128]
        ka = jnp.max(jnp.abs(kk).reshape(CK // 8, 8, D), axis=0)
        return ka if kabs is None else jnp.maximum(kabs, ka)

    ot_v[...] = jnp.zeros_like(ot_v)
    x_copy(0).wait()
    xn = ln1_step(0)
    w_copy(1).wait()
    kabs = None
    kk_prev = None
    for s in range(NC):
        if (s + 1) * CK in XSPLIT[1:-1]:
            x_copy(XSPLIT.index((s + 1) * CK)).wait()
        if s == WQV_STEP:
            w_copy(0).wait()
            w_copy(2).wait()
            wg_copy.start()
            wu_copy.start()
            wd_copy.start()
            wqvt_v[pl.ds(0, D), :] = wqkv_v[:, pl.ds(0, D)].T
            wqvt_v[pl.ds(D, D), :] = wqkv_v[:, pl.ds(2 * D, D)].T
        if kk_prev is not None:
            kabs = k_store(s - 1, kk_prev, kabs)
        xn_next = ln1_step(s + 1) if s + 1 < NC else None
        kk_prev = jnp.dot(xn, wqkv_v[:, pl.ds(D, D)], preferred_element_type=F32)
        xn = xn_next
    kabs = k_store(NC - 1, kk_prev, kabs)

    def qv_block(b, carry):
        vabs, qsum = carry
        rows = pl.ds(pl.multiple_of(b * TQ, TQ), TQ)
        xn = xn_v[rows, :]
        qs = []
        for r0 in range(0, D, 128):
            qt = lax.dot_general(wqvt_v[pl.ds(r0, 128), :], xn, NT,
                                 preferred_element_type=F32) * QSCALE
            qt_v[pl.ds(r0, 128), rows] = qt.astype(BF16)
            qs.append(jnp.sum(jnp.abs(qt).reshape(GH, DH, TQ), axis=1))
        for jj in range(GH // NQ):
            j = b * (GH // NQ) + jj
            q0 = qt_v[pl.ds(pl.multiple_of(j * DH, DH), DH), pl.ds(0, TQ)].astype(F32)
            for cb in range(NB):
                qb_v[j, cb] = jnp.broadcast_to(
                    q0[:, None, cb * 128:(cb + 1) * 128], (DH, 8, 128))
        for r0 in range(0, D, 128):
            vt = lax.dot_general(wqvt_v[pl.ds(D + r0, 128), :], xn, NT,
                                 preferred_element_type=F32)
            vt_v[pl.ds(r0, 128), rows] = vt.astype(BF16)
            vabs = jnp.maximum(vabs, jnp.max(jnp.abs(vt).reshape(16, 8, TQ), axis=0))
        ncb = NC // NQ
        for g in range(KPRE):
            kk = jnp.concatenate(
                [k_v[g, pl.ds(pl.multiple_of((b * ncb + c) * CK, CK), NV), :]
                 for c in range(ncb)], axis=0).astype(F32)
            for d0 in range(0, 128, DH):
                kb_v[g, pl.ds(b * ncb, ncb), pl.ds(d0, DH)] = _lane_replicate(kk, d0, ncb)
        return vabs, jnp.maximum(qsum, jnp.concatenate(qs, axis=0))

    vabs, qsum = lax.fori_loop(
        0, NQ, qv_block, (jnp.zeros((8, TQ), F32), jnp.zeros((H, TQ), F32)), unroll=2)

    bound = jnp.max(qsum) * jnp.max(kabs) * 1.02
    fast = jnp.logical_and(bound <= SCORE_LIMIT, jnp.max(vabs) <= V_LIMIT)
    wo_copy.wait()
    wr_copy.wait()

    def out_proj(t, o_rows, r0, nrows):
        rows = pl.ds(pl.multiple_of((t // NG) * TQ + r0, PR), nrows)
        wo_g = wo_v[pl.ds(pl.multiple_of((t % NG) * 128, 128), 128), :]
        h_v[rows, :] = h_v[rows, :] + jnp.dot(o_rows, wo_g, preferred_element_type=F32)

    def ln2_part(p):
        rows = pl.ds(pl.multiple_of(p * PR, PR), PR)
        h = h_v[rows, :]
        hn = _layernorm(h)
        hn_v[rows, :] = hn
        out_v[rows, :] = (h + hn).astype(BF16)
        t = hn * wr_v[pl.ds(0, D)].astype(F32).reshape(1, D)
        t = (t[:, 0:128] + t[:, 128:256]) + (t[:, 256:384] + t[:, 384:512])
        r_v[pl.ds(p, 1), :] = jnp.sum(t.T, axis=0, keepdims=True)

    def out_copy(p):
        rows = pl.ds(pl.multiple_of(p * PR, PR), PR)
        return pltpu.make_async_copy(out_v.at[rows, :], out_hbm.at[rows, :],
                                     out_sems.at[p])

    def head_weights(g, j, cols):
        q = qt_v[pl.ds(pl.multiple_of(g * 128 + j * DH, DH), DH), cols]
        parts = []
        if j > 0:
            parts.append(jnp.zeros((j * DH, TQ), BF16))
        parts.append(q)
        if j < GH - 1:
            parts.append(jnp.zeros(((GH - 1 - j) * DH, TQ), BF16))
        return jnp.concatenate(parts, axis=0)

    def vpu_scores(kb, groups, j, c):
        res = []
        prev = None
        for b in range(NB):
            keys = kb[groups[b], c, pl.ds(j * DH, DH)].reshape(DH, NV // 8, 8, 128)
            terms = keys * qb_v[j, b][:, None]
            cur = prev
            for d in range(DH):
                cur = terms[d] if cur is None else cur + terms[d]
            res.append(cur if prev is None else cur - prev)
            prev = cur
        return jnp.concatenate(res, axis=2).reshape(NV, TQ)

    def fast_iter(t, first):
        g = t % NG
        cols = pl.ds(pl.multiple_of((t // NG) * TQ, TQ), TQ)
        o_prev = ot_v[...].T
        if first:
            kb = kb_v.at[pl.ds(g, KPRE + 1)]
            groups = [0] * NB
            kk = k32_v[g]
            for d0 in range(0, 128, DH):
                kb[KPRE, :, pl.ds(d0, DH)] = _lane_replicate(kk, d0, NC)
        else:
            kb = kb_v
            groups = [(t + NG * b) % NG for b in range(NB)]
            ln2_part(jnp.maximum(t - PLAG, 0))
        st = {}

        def q_refill(j, c, tie):
            if c % 2:
                return
            js = (j - 1) % GH
            tn = t if j == 0 else jnp.minimum(t + 1, NIT - 1)
            b, d0 = c // 4, (c % 4) * 4
            qn = qt_v[pl.ds(pl.multiple_of((tn % NG) * 128 + js * DH, DH), DH),
                      pl.ds(pl.multiple_of((tn // NG) * TQ + b * 128, 128), 128)]
            qn = qn.astype(F32)[d0:d0 + 8] + tie * 0.0
            qb_v[js, b, pl.ds(d0, 8)] = jnp.stack(
                [jnp.broadcast_to(qn[d:d + 1], (8, 128)) for d in range(8)])

        def stage_a(j, c):
            if c == 0:
                st[j] = dict(w=head_weights(g, j, cols))
            s = jnp.dot(k_v[g, pl.ds(c * CK + NV, NM), :], st[j]['w'],
                        preferred_element_type=F32)
            p = jnp.exp2(s)
            lc = jnp.sum(p.reshape(NM // 8, 8, TQ), axis=0)
            pv = jnp.exp2(vpu_scores(kb, groups, j, c))
            lc = lc + jnp.sum(pv.reshape(NV // 8, 8, TQ), axis=0)
            st[j]['l'] = lc if c == 0 else lc + st[j]['l']
            return jnp.concatenate([pv, p], axis=0)

        def stage_b(j, c, p):
            hrows = pl.ds(pl.multiple_of(g * 128 + j * DH, DH), DH)
            vt = vt_v[hrows, pl.ds(c * CK, CK)]
            oc = jnp.concatenate(
                [lax.dot_general(vt, p[:, :128].astype(BF16), NN, preferred_element_type=F32),
                 lax.dot_general(vt, p[:, 128:], NN, preferred_element_type=F32)], axis=1)
            q_refill(j, c, oc[8:, TQ - 128:])
            st[j]['o'] = oc if c == 0 else oc + st[j]['o']
            if c == NC - 1:
                lsum = jnp.sum(st[j]['l'], axis=0, keepdims=True)
                inv = pl.reciprocal(lsum, approx=True)
                inv = inv * (2.0 - lsum * inv)
                ot_v[pl.ds(j * DH, DH), :] = (st[j]['o'] * inv).astype(BF16)

        seq = [(j, c) for j in range(GH) for c in range(NC)]
        ps = {}
        for i in range(len(seq) + LAG):
            if i < len(seq):
                ps[i] = stage_a(*seq[i])
            if i == len(seq):
                out_proj(jnp.maximum(t - 1, 0), o_prev[:OP1], 0, OP1)
            if i >= LAG:
                stage_b(*seq[i - LAG], ps.pop(i - LAG))
        out_proj(jnp.maximum(t - 1, 0), o_prev[OP1:], OP1, TQ - OP1)

        if not first:
            @pl.when(t >= PLAG)
            def _():
                out_copy(t - PLAG).start()

    def fast_first(t, carry):
        fast_iter(t, True)
        return carry

    def fast_rest(t, carry):
        fast_iter(t, False)
        return carry

    def slow_iter(t, carry):
        g = t % NG
        cols = pl.ds(pl.multiple_of((t // NG) * TQ, TQ), TQ)
        op_v[...] = ot_v[...].T

        def proj(i, c2):
            r0 = pl.multiple_of(i * PR, PR)
            out_proj(jnp.maximum(t - 1, 0), op_v[pl.ds(r0, PR), :], r0, PR)
            return c2
        lax.fori_loop(0, TQ // PR, proj, 0)
        ln2_part(jnp.maximum(t - PLAG, 0))
        row_head = lax.broadcasted_iota(jnp.int32, (128, TQ), 0) // DH

        def head(j, c2):
            qt = qt_v[pl.ds(pl.multiple_of(g * 128, 128), 128), cols]
            w = jnp.where(row_head == j, qt, jnp.zeros_like(qt))
            hrows = pl.ds(pl.multiple_of(g * 128 + j * DH, DH), DH)

            def scores(c, m):
                keys = pl.ds(pl.multiple_of(c * CK, CK), CK)
                s = jnp.dot(k_v[g, keys, :], w, preferred_element_type=F32)
                s_v[keys, :] = s
                return jnp.maximum(m, jnp.max(s.reshape(CK // 8, 8, TQ), axis=0))
            m = lax.fori_loop(0, NC, scores, jnp.full((8, TQ), -jnp.inf, F32))
            m = jnp.max(m, axis=0, keepdims=True)

            def values(c, lo):
                keys = pl.ds(pl.multiple_of(c * CK, CK), CK)
                p = jnp.exp2(s_v[keys, :] - m)
                lc = jnp.sum(p.reshape(CK // 8, 8, TQ), axis=0)
                oc = lax.dot_general(vt_v[hrows, keys], p, NN, preferred_element_type=F32)
                return lo[0] + lc, lo[1] + oc
            l, o = lax.fori_loop(
                0, NC, values, (jnp.zeros((8, TQ), F32), jnp.zeros((DH, TQ), F32)))
            lsum = jnp.sum(l, axis=0, keepdims=True)
            ot_v[pl.ds(pl.multiple_of(j * DH, DH), DH), :] = (o / lsum).astype(BF16)
            return c2
        lax.fori_loop(0, GH, head, 0)

        @pl.when(t >= PLAG)
        def _():
            out_copy(t - PLAG).start()
        return carry

    @pl.when(fast)
    def _():
        lax.fori_loop(0, NG - KPRE, fast_first, 0)
        lax.fori_loop(NG - KPRE, NIT, fast_rest, 0)

    @pl.when(jnp.logical_not(fast))
    def _():
        lax.fori_loop(0, NIT, slow_iter, 0)

    wg_copy.wait()
    wu_copy.wait()
    wd_copy.wait()
    for p in range(NIT - PLAG - 1):
        out_copy(p).wait()
    o_last = ot_v[...].T
    for p in range(NIT - PLAG, NP):
        r0 = p * PR - (NQ - 1) * TQ
        if r0 >= 0:
            out_proj(NIT - 1, o_last[r0:r0 + PR], r0, PR)
        ln2_part(p)
    for p in range(NIT - PLAG, NP):
        out_copy(p).start()

    def all_max(v):
        return jnp.max(jnp.max(v, axis=0, keepdims=True), axis=1, keepdims=True)

    def all_min(v):
        return jnp.min(jnp.min(v, axis=0, keepdims=True), axis=1, keepdims=True)

    r = r_v[pl.ds(0, NP), :]
    pos = (lax.broadcasted_iota(jnp.int32, (NP, PR), 0) * PR
           + lax.broadcasted_iota(jnp.int32, (NP, PR), 1))
    m1 = all_max(r)
    p1 = jnp.minimum(all_min(jnp.where(r == m1, pos, S)), S - 1)
    r2 = jnp.where(pos == p1, -jnp.inf, r)
    m2 = all_max(r2)
    p2 = jnp.minimum(all_min(jnp.where(r2 == m2, pos, S)), S - 1)
    i1 = p1[0, 0]
    i2 = p2[0, 0]

    row16 = lax.broadcasted_iota(jnp.int32, (SLAB, D), 0)
    xs = jnp.where(row16 == 0, hn_v[pl.ds(i1, 1), :], hn_v[pl.ds(i2, 1), :]).astype(BF16)
    gate = jnp.dot(xs, wg_v[...], preferred_element_type=F32)
    up = jnp.dot(xs, wu_v[...], preferred_element_type=F32)
    act = (gate * jax.nn.sigmoid(gate) * up).astype(BF16)
    y = jnp.dot(act, wd_v[...], preferred_element_type=F32)
    y = y * jax.nn.sigmoid(jnp.where(row16 == 0, m1, m2))
    y1 = y[0:1]
    y2 = y[1:2]

    for p in range(NIT - PLAG - 1, NP):
        out_copy(p).wait()

    def patch(slot, idx):
        base = pl.multiple_of((idx // SLAB) * SLAB, SLAB)
        rows = pl.ds(base, SLAB)
        rid = row16 + base
        upd = jnp.where(rid == i1, y1, 0.0) + jnp.where(rid == i2, y2, 0.0)
        slab_v[slot] = (h_v[rows, :] + (hn_v[rows, :] + upd)).astype(BF16)
        return pltpu.make_async_copy(slab_v.at[slot], out_hbm.at[rows, :],
                                     patch_sems.at[slot])

    cp1 = patch(0, i1)
    cp1.start()

    @pl.when(i1 // SLAB != i2 // SLAB)
    def _():
        cp2 = patch(1, i2)
        cp2.start()
        cp2.wait()

    cp1.wait()


@jax.jit
def pallas_sequential_preLN__mha_block__moe_arch_mod__prompt_kernel(
    A_x: jax.Array,
    A_wqkv: jax.Array,
    A_wo: jax.Array,
    B_x: jax.Array,
    B_w_r: jax.Array,
    B_w_gate: jax.Array,
    B_w_up: jax.Array,
    B_w_down: jax.Array,
):
    del B_x
    any_spec = pl.BlockSpec(memory_space=pl.ANY)
    out = pl.pallas_call(
        _kernel,
        out_shape=jax.ShapeDtypeStruct((S, D), BF16),
        in_specs=[any_spec] * 7,
        out_specs=any_spec,
        scratch_shapes=[
            pltpu.VMEM((S, D), BF16),
            pltpu.VMEM((D, 3 * D), BF16),
            pltpu.VMEM((D, S), BF16),
            pltpu.VMEM((D, S), BF16),
            pltpu.VMEM((GH, NB, DH, 8, 128), F32),
            pltpu.VMEM((NG, NC, 128, NV, 128), F32),
            pltpu.VMEM((NG, S, 128), BF16),
            pltpu.VMEM((NG - KPRE, NC * NV, 128), F32),
            pltpu.VMEM((S, D), BF16),
            pltpu.VMEM((2 * D, D), BF16),
            pltpu.VMEM((S, D), F32),
            pltpu.VMEM((D, D), BF16),
            pltpu.VMEM((16 * D,), BF16),
            pltpu.VMEM((128, TQ), BF16),
            pltpu.VMEM((2 * NP, PR), F32),
            pltpu.VMEM((TQ, 128), BF16),
            pltpu.VMEM((2, SLAB, D), BF16),
            pltpu.VMEM((D, F), BF16),
            pltpu.VMEM((D, F), BF16),
            pltpu.VMEM((F, D), BF16),
            pltpu.VMEM((S, TQ), F32),
            pltpu.VMEM((S, D), F32),
            pltpu.VMEM((S, D), BF16),
            pltpu.SemaphoreType.DMA((NXS + 8,)),
            pltpu.SemaphoreType.DMA((NP,)),
            pltpu.SemaphoreType.DMA((2,)),
        ],
        compiler_params=pltpu.CompilerParams(vmem_limit_bytes=120 * 1024 * 1024),
    )(A_x.reshape(S, D), A_wqkv, A_wo, B_w_r, B_w_gate, B_w_up, B_w_down)
    return out.reshape(1, S, D)
```
